```python
import os as _os
_os.environ.setdefault("JAX_PLATFORMS", "cpu")
import jax
import jax.numpy as jnp

def _softmax(x, axis=-1):
    return jax.nn.softmax(x, axis=axis)
def _gelu(x):
    return jax.nn.gelu(x, approximate=True)
def _silu(x):
    return jax.nn.silu(x)
def _sigmoid(x):
    return jax.nn.sigmoid(x)
def _layernorm(x, axis=-1, eps=1e-5):
    m = jnp.mean(x, axis=axis, keepdims=True)
    v = jnp.var(x, axis=axis, keepdims=True)
    return (x - m) / jnp.sqrt(v + eps)
def _scatter_add(tgt, idx, src, axis=0):
    return tgt.at[idx].add(src)
def _segment_sum(src, seg, n):
    return jax.ops.segment_sum(src, seg, n)
class _Rng:
    def __init__(self, key):
        self._k = key
    def _next(self):
        self._k, sub = jax.random.split(self._k)
        return sub
    def normal(self, shape):
        return jax.random.normal(self._next(), shape, dtype=jnp.bfloat16)
    def randint(self, lo, hi, shape):
        return jax.random.randint(self._next(), shape, lo, hi, dtype=jnp.int32)
    def uniform(self, shape, lo=0.0, hi=1.0):
        return jax.random.uniform(self._next(), shape, jnp.bfloat16, lo, hi)
    def permutation(self, n):
        return jax.random.permutation(self._next(), n)


kernel_name = 'gated_mix__grouped_kv_mqa__glu_gated_reglu__prompt'

def setup_inputs():
    _rng = _Rng(jax.random.key(int.from_bytes(__import__("os").urandom(4), "little")))
    _w = (lambda a: (lambda t: t.astype(jnp.bfloat16) if jnp.issubdtype(t.dtype, jnp.floating) else t)(jnp.asarray(a)))
    def _A_setup():
        B, S, D, H = 1, 2048, 640, 32
        Dh = D // H
        return {
            "x": _w((lambda *s: _rng.normal(s) * 0.05)(B, S, D)),
            "wq": _w((lambda *s: _rng.normal(s) * 0.2)(D, H * Dh)),
            "wk": _w((lambda *s: _rng.normal(s) * 0.2)(D, Dh)),
            "wv": _w((lambda *s: _rng.normal(s) * 0.05)(D, Dh)),
            "wo": _w((lambda *s: _rng.normal(s) * 0.05)(H * Dh, D)),
        }
    _A_in = _A_setup()

    def _B_setup():
        B, S, D, F = 1, 2048, 640, 1536
        return {
            "x": _w((lambda *s: _rng.normal(s) * 0.05)(B, S, D)),
            "W_gate": _w((lambda *s: _rng.normal(s) * 0.4)(D, F) * (2.0 / D) ** 0.5),
            "W_up": _w((lambda *s: _rng.normal(s) * 0.4)(D, F) * (2.0 / D) ** 0.5),
            "W_down": _w((lambda *s: _rng.normal(s) * 0.4)(F, D) * (1.0 / F) ** 0.5),
        }
    _B_in = _B_setup()

    return {
        "A_x": _A_in["x"],
        "A_wq": _A_in["wq"],
        "A_wk": _A_in["wk"],
        "A_wv": _A_in["wv"],
        "A_wo": _A_in["wo"],
        "B_x": _B_in["x"],
        "B_W_gate": _B_in["W_gate"],
        "B_W_up": _B_in["W_up"],
        "B_W_down": _B_in["W_down"],
        "gate_w": _w((lambda *s: _rng.normal(s) * 0.05)(640) * 16.0),
    }

def reference(A_x, A_wq, A_wk, A_wv, A_wo, B_x, B_W_gate, B_W_up, B_W_down, gate_w):
    def _A_ref(x, wq, wk, wv, wo):
        B, S, D = x.shape
        H = 32
        Dh = D // H
        q = (lambda x, *d: x.transpose(*d))((x @ wq).reshape(B, S, H, Dh), 0, 2, 1, 3)
        k = x @ wk
        v = x @ wv
        scores = jnp.einsum("bhqd,bkd->bhqk", q, k) * (Dh ** -0.5)
        p = _softmax(scores, axis=-1)
        o = jnp.einsum("bhqk,bkd->bhqd", p, v)
        return (lambda x, *d: x.transpose(*d))(o, 0, 2, 1, 3).reshape(B, S, H * Dh) @ wo

    def _B_ref(x, W_gate, W_up, W_down):
        gate = jnp.einsum("bsd,df->bsf", x, W_gate)
        up = jnp.einsum("bsd,df->bsf", x, W_up)
        gate = gate * (lambda x, dt: x.astype(dt))(gate > 0, gate.dtype)
        h = gate * up
        return jnp.einsum("bsf,fd->bsd", h, W_down)

    x = A_x
    g = _sigmoid((x * gate_w).sum(-1, keepdims=True))
    a = _A_ref(x, A_wq, A_wk, A_wv, A_wo)
    b = _B_ref(x, B_W_gate, B_W_up, B_W_down)
    return g * a + (1 - g) * b
```

```python
import functools
import jax
import jax.numpy as jnp
from jax import lax
import jax.experimental.pallas as pl
import jax.experimental.pallas.tpu as pltpu

S, D, H, DH, F = 2048, 640, 32, 20, 1536
W = 24
LOG2E = 1.4426950408889634
f32, bf16 = jnp.float32, jnp.bfloat16
NT = (((1,), (1,)), ((), ()))


def make_kernel(tq, tk, pairs_per_iter):
    nc = S // tk

    def kernel(x_ref, wq_ref, wkT_ref, wvT_ref, wo_ref, wg_ref, wu_ref, wd_ref, gw_ref,
               o_ref, k_ref, vT_ref, wqT_ref, qT_ref, oT_ref, s0_ref, s1_ref, m0_ref, m1_ref):
        step = pl.program_id(0)

        @pl.when(step == 0)
        def _prologue():
            x = x_ref[...]
            r = lax.broadcasted_iota(jnp.int32, (128, DH), 0)
            c = lax.broadcasted_iota(jnp.int32, (128, DH), 1)
            Rk = jnp.where((r == c) | (r == c + 36), 1.0, 0.0).astype(bf16)
            wkT_all = jnp.dot(Rk, wkT_ref[...], preferred_element_type=f32).astype(bf16)
            k4 = lax.dot_general(x, wkT_all, NT, preferred_element_type=f32)
            k_ref[0] = k4[:, 0:W].astype(bf16)
            k_ref[1] = k4[:, 32:32 + W].astype(bf16)
            r = lax.broadcasted_iota(jnp.int32, (2 * W, DH), 0)
            c = lax.broadcasted_iota(jnp.int32, (2 * W, DH), 1)
            Rv = jnp.where((r == c) | (r == c + 28), 1.0, 0.0).astype(bf16)
            wvT_all = jnp.dot(Rv, wvT_ref[...], preferred_element_type=f32).astype(bf16)
            vT = lax.dot_general(wvT_all, x, NT, preferred_element_type=f32)
            row = lax.broadcasted_iota(jnp.int32, (2 * W, S), 0)
            ones = (row == 20) | (row == 24)
            vT_ref[...] = jnp.where(ones, 1.0, vT.astype(bf16).astype(f32))
            wqT_ref[...] = wq_ref[...].astype(f32).T.astype(bf16)

        row0 = pl.multiple_of(step * tq, tq)
        xb = x_ref[pl.ds(row0, tq), :]
        qT = lax.dot_general(wqT_ref[...], xb, NT, preferred_element_type=f32)
        qT_ref[...] = qT * (DH ** -0.5 * LOG2E)

        s_refs = (s0_ref, s1_ref)
        m_refs = (m0_ref, m1_ref)
        lrow = (20, 0)

        def q_of(i, e):
            start = 40 * i + 16 * e
            if not isinstance(start, int):
                start = pl.multiple_of(start, 8)
            return qT_ref[pl.ds(start, W), :].astype(bf16)

        def unit(a, b):
            if a is not None:
                qa = q_of(*a)
                ea = a[1]
                macc = None
            if b is not None:
                mb = m_refs[b][0:1, :]
                acc = None
            for c in range(nc):
                rows = pl.ds(c * tk, tk)
                if a is not None:
                    s = jnp.dot(k_ref[ea, rows, :], qa, preferred_element_type=f32)
                    s_refs[ea][rows, :] = s
                    mc = jnp.max(s.reshape(tk // 8, 8, tq), axis=0)
                    macc = mc if macc is None else jnp.maximum(macc, mc)
                if b is not None:
                    p = jnp.exp2(s_refs[b][rows, :] - mb).astype(bf16)
                    pv = jnp.dot(vT_ref[W * b:W * b + W, rows], p, preferred_element_type=f32)
                    acc = pv if acc is None else acc + pv
            if a is not None:
                m_refs[ea][...] = jnp.broadcast_to(jnp.max(macc, axis=0, keepdims=True), (8, tq))
            if b is not None:
                return acc * (1.0 / acc[lrow[b]:lrow[b] + 1])
            return None

        def store_pair(i, oe, oo):
            base = 40 * i
            if not isinstance(base, int):
                base = pl.multiple_of(base, 8)
            r8 = lax.broadcasted_iota(jnp.int32, (8, tq), 0)
            oT_ref[pl.ds(base, 16), :] = oe[0:16]
            oT_ref[pl.ds(base + 16, 8), :] = jnp.where(r8 < 4, oe[16:24], oo[0:8])
            oT_ref[pl.ds(base + 24, 16), :] = oo[8:24]

        def pair(i):
            oe = unit((i, 1), 0)
            oo = unit((i + 1, 0), 1)
            store_pair(i, oe, oo)

        unit((0, 0), None)
        npairs = H // 2
        n_loop = (npairs - 1) // pairs_per_iter

        def body(it, carry):
            for u in range(pairs_per_iter):
                pair(it * pairs_per_iter + u)
            return carry

        lax.fori_loop(0, n_loop, body, 0)
        for i in range(n_loop * pairs_per_iter, npairs - 1):
            pair(i)
        i_last = npairs - 1
        oe = unit((i_last, 1), 0)
        oo = unit(None, 1)
        store_pair(i_last, oe, oo)

        gate = jnp.dot(xb, wg_ref[...], preferred_element_type=f32)
        up = jnp.dot(xb, wu_ref[...], preferred_element_type=f32)
        h = (jnp.maximum(gate, 0.0) * up).astype(bf16)
        b_out = jnp.dot(h, wd_ref[...], preferred_element_type=f32)
        o_all = oT_ref[...].T.astype(bf16)
        a_out = jnp.dot(o_all, wo_ref[...], preferred_element_type=f32)
        logit = jnp.sum(xb.astype(f32) * gw_ref[...].astype(f32), axis=-1, keepdims=True)
        g = jax.nn.sigmoid(logit)
        o_ref[...] = (g * a_out + (1.0 - g) * b_out).astype(o_ref.dtype)
    return kernel


def build(tq=512, tk=256, ppi=1):
    @jax.jit
    def run(A_x, A_wq, A_wk, A_wv, A_wo, B_x, B_W_gate, B_W_up, B_W_down, gate_w):
        x = A_x.reshape(S, D)
        gw = gate_w.reshape(1, D)
        full = lambda shape: pl.BlockSpec(shape, lambda i: (0,) * len(shape))
        out = pl.pallas_call(
            make_kernel(tq, tk, ppi),
            grid=(S // tq,),
            in_specs=[full((S, D)), full((D, D)), full((DH, D)), full((DH, D)), full((D, D)),
                      full((D, F)), full((D, F)), full((F, D)), full((1, D))],
            out_specs=pl.BlockSpec((tq, D), lambda i: (i, 0)),
            out_shape=jax.ShapeDtypeStruct((S, D), bf16),
            scratch_shapes=[
                pltpu.VMEM((2, S, W), bf16),
                pltpu.VMEM((2 * W, S), f32),
                pltpu.VMEM((D, D), bf16),
                pltpu.VMEM((D, tq), f32),
                pltpu.VMEM((D, tq), f32),
                pltpu.VMEM((S, tq), f32),
                pltpu.VMEM((S, tq), f32),
                pltpu.VMEM((8, tq), f32),
                pltpu.VMEM((8, tq), f32),
            ],
            compiler_params=pltpu.CompilerParams(
                dimension_semantics=("arbitrary",), vmem_limit_bytes=100 * 1024 * 1024),
        )(x, A_wq, A_wk.T, A_wv.T, A_wo, B_W_gate, B_W_up, B_W_down, gw)
        return out.reshape(1, S, D)
    return run


_RUN = build(tq=512,tk=128,ppi=3)


@jax.jit
def pallas_gated_mix__grouped_kv_mqa__glu_gated_reglu__prompt_kernel(
    A_x: jax.Array,
    A_wq: jax.Array,
    A_wk: jax.Array,
    A_wv: jax.Array,
    A_wo: jax.Array,
    B_x: jax.Array,
    B_W_gate: jax.Array,
    B_W_up: jax.Array,
    B_W_down: jax.Array,
    gate_w: jax.Array,
):
    return _RUN(A_x, A_wq, A_wk, A_wv, A_wo, B_x, B_W_gate, B_W_up, B_W_down, gate_w)
```

```python
import functools
import jax
import jax.numpy as jnp
from jax import lax
import jax.experimental.pallas as pl
import jax.experimental.pallas.tpu as pltpu

S, D, H, DH, F = 2048, 640, 32, 20, 1536
W = 24
LOG2E = 1.4426950408889634
f32, bf16 = jnp.float32, jnp.bfloat16
NT = (((1,), (1,)), ((), ()))
TK = 128
NC = S // TK


def make_kernel(tq, delta, unroll, nxc):
    xc = S // nxc

    def kernel(x_hbm, wq_hbm, wkT_hbm, wvT_hbm, wo_hbm, wg_hbm, wu_hbm, wd_hbm, gw_hbm,
               o_ref,
               x_ref, wq_ref, wkT_ref, wvT_ref, wo_ref, wg_ref, wu_ref, wd_ref, gw_ref, sems,
               k_ref, vT_ref, wqT_ref, qT_ref, oT_ref, s0_ref, s1_ref, m0_ref, m1_ref,
               ma0_ref, ma1_ref):
        step = pl.program_id(0)

        def x_copy(j):
            return pltpu.make_async_copy(x_hbm.at[pl.ds(j * xc, xc)], x_ref.at[pl.ds(j * xc, xc)], sems.at[j])

        small = [(wkT_hbm, wkT_ref), (wvT_hbm, wvT_ref), (gw_hbm, gw_ref), (wq_hbm, wq_ref)]
        late = [(wg_hbm, wg_ref), (wu_hbm, wu_ref), (wd_hbm, wd_ref), (wo_hbm, wo_ref)]

        def small_copy(j):
            return pltpu.make_async_copy(small[j][0], small[j][1], sems.at[nxc + j])

        def late_copy(j):
            return pltpu.make_async_copy(late[j][0], late[j][1], sems.at[nxc + 4 + j])

        @pl.when(step == 0)
        def _prologue():
            small_copy(0).start()
            small_copy(1).start()
            for j in range(nxc):
                x_copy(j).start()
            small_copy(3).start()
            small_copy(2).start()
            for j in range(4):
                late_copy(j).start()
            small_copy(0).wait()
            small_copy(1).wait()
            r = lax.broadcasted_iota(jnp.int32, (128, DH), 0)
            c = lax.broadcasted_iota(jnp.int32, (128, DH), 1)
            Rk = jnp.where((r == c) | (r == c + 36), 1.0, 0.0).astype(bf16)
            wkT_all = jnp.dot(Rk, wkT_ref[...], preferred_element_type=f32).astype(bf16)
            r = lax.broadcasted_iota(jnp.int32, (2 * W, DH), 0)
            c = lax.broadcasted_iota(jnp.int32, (2 * W, DH), 1)
            Rv = jnp.where((r == c) | (r == c + 28), 1.0, 0.0).astype(bf16)
            wvT_all = jnp.dot(Rv, wvT_ref[...], preferred_element_type=f32).astype(bf16)
            row = lax.broadcasted_iota(jnp.int32, (2 * W, xc), 0)
            ones = (row == 20) | (row == 24)
            for j in range(nxc):
                x_copy(j).wait()
                rows = pl.ds(j * xc, xc)
                x = x_ref[rows, :]
                k4 = lax.dot_general(x, wkT_all, NT, preferred_element_type=f32)
                k_ref[0, rows, :] = k4[:, 0:W].astype(bf16)
                k_ref[1, rows, :] = k4[:, 32:32 + W].astype(bf16)
                vT = lax.dot_general(wvT_all, x, NT, preferred_element_type=f32)
                vT_ref[:, rows] = jnp.where(ones, 1.0, vT.astype(bf16).astype(f32))
            small_copy(3).wait()
            small_copy(2).wait()
            wqT_ref[...] = wq_ref[...].astype(f32).T.astype(bf16)

        row0 = pl.multiple_of(step * tq, tq)
        xb = x_ref[pl.ds(row0, tq), :]
        qT = lax.dot_general(wqT_ref[...], xb, NT, preferred_element_type=f32)
        qT_ref[...] = qT * (DH ** -0.5 * LOG2E)

        s_refs = (s0_ref, s1_ref)
        m_refs = (m0_ref, m1_ref)
        ma_refs = (ma0_ref, ma1_ref)
        lrow = (20, 0)

        def mult(v, k):
            return v if isinstance(v, int) else pl.multiple_of(v, k)

        def a_slot(st, pi, e, c):
            key = ('A', e)
            if key not in st:
                qwin = qT_ref[pl.ds(mult(40 * pi + 16 * e, 8), W), :]
                st[key] = dict(qa=qwin.astype(bf16), macc=None)
                if c > 0:
                    st[key]['macc'] = ma_refs[e][...]
            a = st[key]
            rows = pl.ds(c * TK, TK)
            s = jnp.dot(k_ref[e, rows, :], a['qa'], preferred_element_type=f32)
            s_refs[e][rows, :] = s
            mc = jnp.max(s.reshape(TK // 8, 8, tq), axis=0)
            a['macc'] = mc if a['macc'] is None else jnp.maximum(a['macc'], mc)
            if c == NC - 1:
                m_refs[e][...] = jnp.broadcast_to(jnp.max(a['macc'], axis=0, keepdims=True), (8, tq))
                del st[key]

        def a_flush(st):
            for key in [k for k in st if k[0] == 'A']:
                ma_refs[key[1]][...] = st[key]['macc']
                del st[key]

        def b_slot(st, pi, e, c):
            key = ('B', e)
            if key not in st:
                st[key] = dict(mb=m_refs[e][0:1, :], acc=None)
            b = st[key]
            rows = pl.ds(c * TK, TK)
            p = jnp.exp2(s_refs[e][rows, :] - b['mb']).astype(bf16)
            pv = jnp.dot(vT_ref[W * e:W * e + W, rows], p, preferred_element_type=f32)
            b['acc'] = pv if b['acc'] is None else b['acc'] + pv
            if c == NC - 1:
                acc = b['acc']
                o = acc * (1.0 / acc[lrow[e]:lrow[e] + 1])
                base = mult(40 * pi, 8)
                if e == 0:
                    oT_ref[pl.ds(base, W), :] = o
                else:
                    r8 = lax.broadcasted_iota(jnp.int32, (8, tq), 0)
                    oT_ref[pl.ds(base + 16, 8), :] = jnp.where(r8 < 4, oT_ref[pl.ds(base + 16, 8), :], o[0:8])
                    oT_ref[pl.ds(base + 24, 16), :] = o[8:24]
                del st[key]

        L = NC + delta

        def run_slots(st, i, t_lo, t_hi, do_a=True, do_b=True):
            for t in range(t_lo, t_hi):
                if do_a:
                    u, c = divmod(t, NC)
                    if not (isinstance(i, int) and 2 * i + u >= H):
                        a_slot(st, i + u // 2, u % 2, c)
                if do_b:
                    tb = t - L
                    if not (isinstance(i, int) and 2 * i * NC + tb < 0):
                        u, c = divmod(tb, NC)
                        b_slot(st, i + u // 2, u % 2, c)
            a_flush(st)

        st = {}
        run_slots(st, 0, 0, L, do_b=False)

        n_body = H // 2 - 1
        n_loop = n_body // unroll

        def body(it, carry):
            st = {}
            for u in range(unroll):
                run_slots(st, it * unroll + u, L, L + 2 * NC)
            return carry

        lax.fori_loop(0, n_loop, body, 0)

        @pl.when(step == 0)
        def _wait_late():
            for j in range(4):
                late_copy(j).wait()

        st = {}
        for i in range(n_loop * unroll, n_body + 1):
            run_slots(st, i, L, L + 2 * NC)

        gate = jnp.dot(xb, wg_ref[...], preferred_element_type=f32)
        up = jnp.dot(xb, wu_ref[...], preferred_element_type=f32)
        h = (jnp.maximum(gate, 0.0) * up).astype(bf16)
        b_out = jnp.dot(h, wd_ref[...], preferred_element_type=f32)
        o_all = oT_ref[...].T.astype(bf16)
        a_out = jnp.dot(o_all, wo_ref[...], preferred_element_type=f32)
        xf = x_ref[pl.ds(row0, tq), :].astype(f32)
        gw = gw_ref[...].astype(f32)
        la = xf[:, 0:128] * gw[0:1, :]
        for j in range(1, D // 128):
            la = la + xf[:, 128 * j:128 * (j + 1)] * gw[j:j + 1, :]
        logit = jnp.sum(la, axis=-1, keepdims=True)
        g = jax.nn.sigmoid(logit)
        o_ref[...] = (g * a_out + (1.0 - g) * b_out).astype(o_ref.dtype)
    return kernel


def build(tq=512, delta=2, unroll=1, nxc=4):
    @jax.jit
    def run(A_x, A_wq, A_wk, A_wv, A_wo, B_x, B_W_gate, B_W_up, B_W_down, gate_w):
        x = A_x.reshape(S, D)
        gw = gate_w.reshape(D // 128, 128)
        hbm = pl.BlockSpec(memory_space=pl.ANY)
        out = pl.pallas_call(
            make_kernel(tq, delta, unroll, nxc),
            grid=(S // tq,),
            in_specs=[hbm] * 9,
            out_specs=pl.BlockSpec((tq, D), lambda i: (i, 0)),
            out_shape=jax.ShapeDtypeStruct((S, D), bf16),
            scratch_shapes=[
                pltpu.VMEM((S, D), bf16),
                pltpu.VMEM((D, D), bf16),
                pltpu.VMEM((DH, D), bf16),
                pltpu.VMEM((DH, D), bf16),
                pltpu.VMEM((D, D), bf16),
                pltpu.VMEM((D, F), bf16),
                pltpu.VMEM((D, F), bf16),
                pltpu.VMEM((F, D), bf16),
                pltpu.VMEM((D // 128, 128), bf16),
                pltpu.SemaphoreType.DMA((nxc + 8,)),
                pltpu.VMEM((2, S, W), bf16),
                pltpu.VMEM((2 * W, S), f32),
                pltpu.VMEM((D, D), bf16),
                pltpu.VMEM((D, tq), f32),
                pltpu.VMEM((D, tq), f32),
                pltpu.VMEM((S, tq), f32),
                pltpu.VMEM((S, tq), f32),
                pltpu.VMEM((8, tq), f32),
                pltpu.VMEM((8, tq), f32),
                pltpu.VMEM((8, tq), f32),
                pltpu.VMEM((8, tq), f32),
            ],
            compiler_params=pltpu.CompilerParams(
                dimension_semantics=("arbitrary",), vmem_limit_bytes=100 * 1024 * 1024),
        )(x, A_wq, A_wk.T, A_wv.T, A_wo, B_W_gate, B_W_up, B_W_down, gw)
        return out.reshape(1, S, D)
    return run


_RUN = build(unroll=5)


@jax.jit
def pallas_gated_mix__grouped_kv_mqa__glu_gated_reglu__prompt_kernel(
    A_x: jax.Array,
    A_wq: jax.Array,
    A_wk: jax.Array,
    A_wv: jax.Array,
    A_wo: jax.Array,
    B_x: jax.Array,
    B_W_gate: jax.Array,
    B_W_up: jax.Array,
    B_W_down: jax.Array,
    gate_w: jax.Array,
):
    return _RUN(A_x, A_wq, A_wk, A_wv, A_wo, B_x, B_W_gate, B_W_up, B_W_down, gate_w)
```

```python
import jax
import jax.numpy as jnp
from jax import lax
import jax.experimental.pallas as pl
import jax.experimental.pallas.tpu as pltpu

S, D, H, DH, F = 2048, 640, 32, 20, 1536
W = 24
LOG2E = 1.4426950408889634
f32, bf16, u32 = jnp.float32, jnp.bfloat16, jnp.uint32
NT = (((1,), (1,)), ((), ()))
TK = 128
NC = S // TK
SCORE_BOUND = 60.0
V_HI = 2.0 ** 40
V_LO = 2.0 ** -30


def make_kernel(tq, nxc, vr, vr0, lead, upb, tks):
    xc = S // nxc
    nbody = H // upb
    nvmax = max(sum(vr), sum(vr0))
    last_par = (nbody - 1) % 2

    def vcfg(v):
        nv = sum(v)
        ngroups = nv // 8
        gps = [ngroups // NC + (1 if c < ngroups % NC else 0) for c in range(NC)]
        return dict(vr=v, nv=nv, blk_row=[c * TK + 16 * b for c in range(NC) for b in range(v[c] // 16)],
                    glo=[sum(gps[:c]) for c in range(NC + 1)])

    vu = [max(a, b) for a, b in zip(vr, vr0)]
    kbo = [sum(vu[:c]) for c in range(NC + 1)]
    cfg_loop, cfg_first = vcfg(vr), vcfg(vr0)

    def kb_row(key_row):
        c, r = divmod(key_row, TK)
        return kbo[c] + r

    def kernel(x_hbm, wq_hbm, wkT_hbm, wvT_hbm, wo_hbm, wg_hbm, wu_hbm, wd_hbm, gw_hbm,
               o_ref,
               x_ref, wq_ref, wkT_ref, wvT_ref, wo_ref, wg_ref, wu_ref, wd_ref, gw_ref, sems,
               k_ref, vT_ref, wqT_ref, qT_ref, oT_ref, kb_ref, qb_ref, tok_ref, stat_ref, *p_refs):
        step = pl.program_id(0)

        def x_copy(j):
            return pltpu.make_async_copy(x_hbm.at[pl.ds(j * xc, xc)], x_ref.at[pl.ds(j * xc, xc)], sems.at[j])

        small = [(wkT_hbm, wkT_ref), (wvT_hbm, wvT_ref), (gw_hbm, gw_ref), (wq_hbm, wq_ref)]
        late = [(wg_hbm, wg_ref), (wu_hbm, wu_ref), (wd_hbm, wd_ref), (wo_hbm, wo_ref)]

        def small_copy(j):
            return pltpu.make_async_copy(small[j][0], small[j][1], sems.at[nxc + j])

        def late_copy(j):
            return pltpu.make_async_copy(late[j][0], late[j][1], sems.at[nxc + 4 + j])

        @pl.when(step == 0)
        def _prologue():
            small_copy(0).start()
            small_copy(1).start()
            for j in range(nxc):
                x_copy(j).start()
            small_copy(3).start()
            small_copy(2).start()
            for j in range(4):
                late_copy(j).start()
            small_copy(0).wait()
            small_copy(1).wait()
            r = lax.broadcasted_iota(jnp.int32, (128, DH), 0)
            c = lax.broadcasted_iota(jnp.int32, (128, DH), 1)
            Rk = jnp.where((r == c) | (r == c + 36), 1.0, 0.0).astype(bf16)
            wkT_all = jnp.dot(Rk, wkT_ref[...], preferred_element_type=f32).astype(bf16)
            r = lax.broadcasted_iota(jnp.int32, (2 * W, DH), 0)
            c = lax.broadcasted_iota(jnp.int32, (2 * W, DH), 1)
            Rv = jnp.where((r == c) | (r == c + 28), 1.0, 0.0).astype(bf16)
            wvT_all = jnp.dot(Rv, wvT_ref[...], preferred_element_type=f32).astype(bf16)
            row = lax.broadcasted_iota(jnp.int32, (2 * W, xc), 0)
            ones = (row == 20) | (row == 24)
            kmax = None
            vmax = None
            for j in range(nxc):
                x_copy(j).wait()
                rows = pl.ds(j * xc, xc)
                x = x_ref[rows, :]
                k4 = lax.dot_general(x, wkT_all, NT, preferred_element_type=f32)
                k_ref[0, rows, :] = k4[:, 0:W].astype(bf16)
                k_ref[1, rows, :] = k4[:, 32:32 + W].astype(bf16)
                km = jnp.max(jnp.abs(k4).reshape(xc // 8, 8, 128), axis=0)
                kmax = km if kmax is None else jnp.maximum(kmax, km)
                vT = lax.dot_general(wvT_all, x, NT, preferred_element_type=f32)
                vT_ref[:, rows] = jnp.where(ones, 1.0, vT.astype(bf16).astype(f32))
                vm = jnp.abs(vT[0:W])
                vmax = vm if vmax is None else jnp.maximum(vmax, vm)
            vmx = jnp.max(vmax)
            v_ok = jnp.logical_and(vmx <= V_HI, vmx >= V_LO)
            stat_ref[0] = jnp.where(v_ok, jnp.max(kmax) * (DH * 1.02), jnp.inf)
            if nvmax:
                r = lax.broadcasted_iota(jnp.int32, (W, DH * 128), 0)
                c = lax.broadcasted_iota(jnp.int32, (W, DH * 128), 1)
                E = jnp.where(r == c // 128, 1.0, 0.0).astype(bf16)
                for c in range(NC):
                    if vu[c]:
                        kb_ref[pl.ds(kbo[c], vu[c]), :] = jnp.dot(k_ref[0, pl.ds(c * TK, vu[c]), :], E,
                                                                  preferred_element_type=f32)
            small_copy(3).wait()
            small_copy(2).wait()
            wqT_ref[...] = wq_ref[...].astype(f32).T.astype(bf16)

        row0 = pl.multiple_of(step * tq, tq)
        xb = x_ref[pl.ds(row0, tq), :]
        qT = lax.dot_general(wqT_ref[...], xb, NT, preferred_element_type=f32) * (DH ** -0.5 * LOG2E)
        qT_ref[...] = qT
        qmax = jnp.max(jnp.max(jnp.abs(qT).reshape(D // 8, 8, tq), axis=0))
        fast = qmax * stat_ref[0] <= SCORE_BOUND

        lrow = (20, 0)

        def mult(v, k):
            return v if isinstance(v, int) else pl.multiple_of(v, k)

        def store_head(base, e, o):
            if e == 0:
                oT_ref[pl.ds(base, W), :] = o
            else:
                r8 = lax.broadcasted_iota(jnp.int32, (8, tq), 0)
                oT_ref[pl.ds(base + 16, 8), :] = jnp.where(r8 < 4, oT_ref[pl.ds(base + 16, 8), :], o[0:8])
                oT_ref[pl.ds(base + 24, 16), :] = o[8:24]

        def a_slot(st, cfg, bi, par, u, c):
            e = u % 2
            key = ('A', u)
            buf = upb * par + u
            v, glo, blk_row = cfg['vr'], cfg['glo'], cfg['blk_row']
            if key not in st:
                qwin = qT_ref[pl.ds(mult(20 * upb * bi + 40 * (u // 2) + 16 * e, 8), W), :]
                st[key] = dict(qa=qwin.astype(bf16), val=None, half=None)
                if cfg['nv']:
                    for d in range(DH):
                        qb_ref[u, d] = jnp.broadcast_to(qwin[4 * e + d:4 * e + d + 1, :], (8, tq))
            a = st[key]

            def chain(f):
                a['val'] = f if a['val'] is None else jnp.maximum(a['val'], f)

            lo, n = c * TK + v[c], TK - v[c]
            s = jnp.dot(k_ref[e, pl.ds(lo, n), :], a['qa'], preferred_element_type=f32)
            p_refs[buf][pl.ds(lo // 2, n // 2), :] = pltpu.bitcast(jnp.exp2(s).astype(bf16), u32)
            chain(s[0:8])
            for g in range(glo[c], glo[c + 1]):
                krow = kb_row(blk_row[g // 2] + 8 * (g % 2))
                sv = None
                for d in range(DH):
                    kb = kb_ref[pl.ds(krow, 8), pl.ds(128 * d, 128)]
                    kbt = jnp.concatenate([kb] * (tq // 128), axis=1)
                    t = kbt * qb_ref[u, d]
                    sv = t if sv is None else sv + t
                chain(sv)
                pv = jnp.exp2(sv)
                if g % 2 == 0:
                    a['half'] = pv
                else:
                    pu = pltpu.bitcast(jnp.concatenate([a['half'], pv], axis=0).astype(bf16), u32)
                    p_refs[buf][pl.ds(blk_row[g // 2] // 2, 8), :] = pu
            if c == NC - 1:
                tok_ref[u] = a['val']
                del st[key]

        def b_slot(st, bi, par, u, c):
            e = u % 2
            buf = upb * par + u
            key = ('B', u)
            if key not in st:
                st[key] = dict(val=None)
            b = st[key]
            p = pltpu.bitcast(p_refs[buf][pl.ds(c * TK // 2, TK // 2), :], bf16)
            vt = vT_ref[W * e:W * e + W, pl.ds(c * TK, TK)]
            pv = jnp.dot(vt, p, preferred_element_type=f32)
            b['val'] = pv if b['val'] is None else b['val'] + pv
            if c == NC - 1:
                acc = b['val']
                store_head(mult(20 * upb * bi + 40 * (u // 2), 8), e, acc * (1.0 / acc[lrow[e]:lrow[e] + 1]))
                del st[key]

        def body(cfg, ia, para, ib, parb):
            st = {}
            nb = 0
            nt = upb * NC
            for t in range(nt):
                if ia is not None:
                    a_slot(st, cfg, ia, para, t // NC, t % NC)
                if ib is not None:
                    while nb < nt and nb <= t + lead:
                        b_slot(st, ib, parb, nb // NC, nb % NC)
                        nb += 1
            if ib is not None:
                while nb < nt:
                    b_slot(st, ib, parb, nb // NC, nb % NC)
                    nb += 1

        def dense_tail():
            gate = jnp.dot(xb, wg_ref[...], preferred_element_type=f32)
            up = jnp.dot(xb, wu_ref[...], preferred_element_type=f32)
            h = (jnp.maximum(gate, 0.0) * up).astype(bf16)
            b_out = jnp.dot(h, wd_ref[...], preferred_element_type=f32)
            o_all = oT_ref[...].T.astype(bf16)
            a_out = jnp.dot(o_all, wo_ref[...], preferred_element_type=f32)
            xf = x_ref[pl.ds(row0, tq), :].astype(f32)
            gw = gw_ref[...].astype(f32)
            la = xf[:, 0:128] * gw[0:1, :]
            for j in range(1, D // 128):
                la = la + xf[:, 128 * j:128 * (j + 1)] * gw[j:j + 1, :]
            g = jax.nn.sigmoid(jnp.sum(la, axis=-1, keepdims=True))
            o_ref[...] = (g * a_out + (1.0 - g) * b_out).astype(o_ref.dtype)

        body(cfg_first, 0, 0, None, None)

        @pl.when(step == 0)
        def _wait_late():
            for j in range(4):
                late_copy(j).wait()

        @pl.when(fast)
        def _fast():
            def loop_body(i, carry):
                @pl.when(i % 2 == 0)
                def _():
                    body(cfg_loop, i + 1, 1, i, 0)

                @pl.when(i % 2 == 1)
                def _():
                    body(cfg_loop, i + 1, 0, i, 1)
                return carry

            lax.fori_loop(0, nbody - 1, loop_body, 0)

        @pl.when(jnp.logical_not(fast))
        def _slow():
            def q_of(pi, e):
                return qT_ref[pl.ds(mult(40 * pi + 16 * e, 8), W), :].astype(bf16)

            def scores(e, qa, j):
                r0 = pl.multiple_of(j * tks, tks)
                return r0, jnp.dot(k_ref[e, pl.ds(r0, tks), :], qa, preferred_element_type=f32)

            def pair_body(pi, carry):
                for e in range(2):
                    qa = q_of(pi, e)

                    def chunk(j, mc):
                        m, acc = mc
                        r0, s = scores(e, qa, j)
                        m_new = jnp.maximum(m, jnp.max(s, axis=0, keepdims=True))
                        p = jnp.exp2(s - m_new).astype(bf16)
                        pv = jnp.dot(vT_ref[W * e:W * e + W, pl.ds(r0, tks)], p, preferred_element_type=f32)
                        return m_new, acc * jnp.exp2(m - m_new) + pv

                    m0 = jnp.full((1, tq), -jnp.inf, f32)
                    _, acc = lax.fori_loop(0, S // tks, chunk, (m0, jnp.zeros((W, tq), f32)))
                    store_head(pl.multiple_of(40 * pi, 8), e, acc * (1.0 / acc[lrow[e]:lrow[e] + 1]))
                return carry

            lax.fori_loop(0, (H - upb) // 2, pair_body, 0)
            for u in range(upb):
                e = u % 2
                qa = q_of((H - upb) // 2 + u // 2, e)
                buf = upb * last_par + u

                def row_max(j, m):
                    return jnp.maximum(m, jnp.max(scores(e, qa, j)[1], axis=0, keepdims=True))

                m = lax.fori_loop(0, S // tks, row_max, jnp.full((1, tq), -jnp.inf, f32))

                def write_p(j, carry):
                    r0, s = scores(e, qa, j)
                    p = pltpu.bitcast(jnp.exp2(s - m).astype(bf16), u32)
                    p_refs[buf][pl.ds(pl.multiple_of(j * (tks // 2), tks // 2), tks // 2), :] = p
                    return carry

                lax.fori_loop(0, S // tks, write_p, 0)

        body(None, None, None, nbody - 1, last_par)
        dense_tail()
    return kernel


def build(tq=512, nxc=4, vr=None, vr0=None, lead=-1, upb=4, tks=256):
    if vr is None:
        vr = [16, 0] * 8
    if vr0 is None:
        vr0 = vr

    def run(A_x, A_wq, A_wk, A_wv, A_wo, B_x, B_W_gate, B_W_up, B_W_down, gate_w):
        x = A_x.reshape(S, D)
        gw = gate_w.reshape(D // 128, 128)
        hbm = pl.BlockSpec(memory_space=pl.ANY)
        nvu = sum(max(a, b) for a, b in zip(vr, vr0))
        out = pl.pallas_call(
            make_kernel(tq, nxc, tuple(vr), tuple(vr0), lead, upb, tks),
            grid=(S // tq,),
            in_specs=[hbm] * 9,
            out_specs=pl.BlockSpec((tq, D), lambda i: (i, 0)),
            out_shape=jax.ShapeDtypeStruct((S, D), bf16),
            scratch_shapes=[
                pltpu.VMEM((S, D), bf16),
                pltpu.VMEM((D, D), bf16),
                pltpu.VMEM((DH, D), bf16),
                pltpu.VMEM((DH, D), bf16),
                pltpu.VMEM((D, D), bf16),
                pltpu.VMEM((D, F), bf16),
                pltpu.VMEM((D, F), bf16),
                pltpu.VMEM((F, D), bf16),
                pltpu.VMEM((D // 128, 128), bf16),
                pltpu.SemaphoreType.DMA((nxc + 8,)),
                pltpu.VMEM((2, S, W), bf16),
                pltpu.VMEM((2 * W, S), f32),
                pltpu.VMEM((D, D), bf16),
                pltpu.VMEM((D, tq), f32),
                pltpu.VMEM((D, tq), f32),
                pltpu.VMEM((max(nvu, 8), DH * 128), f32),
                pltpu.VMEM((upb, DH, 8, tq), f32),
                pltpu.VMEM((upb, 8, tq), f32),
                pltpu.SMEM((1,), f32),
            ] + [pltpu.VMEM((S // 2, tq), u32)] * (2 * upb),
            compiler_params=pltpu.CompilerParams(
                dimension_semantics=("arbitrary",), vmem_limit_bytes=120 * 1024 * 1024),
        )(x, A_wq, A_wk.T, A_wv.T, A_wo, B_W_gate, B_W_up, B_W_down, gw)
        return out.reshape(1, S, D)
    return jax.jit(run)


_RUN = build()


@jax.jit
def pallas_gated_mix__grouped_kv_mqa__glu_gated_reglu__prompt_kernel(
    A_x: jax.Array,
    A_wq: jax.Array,
    A_wk: jax.Array,
    A_wv: jax.Array,
    A_wo: jax.Array,
    B_x: jax.Array,
    B_W_gate: jax.Array,
    B_W_up: jax.Array,
    B_W_down: jax.Array,
    gate_w: jax.Array,
):
    return _RUN(A_x, A_wq, A_wk, A_wv, A_wo, B_x, B_W_gate, B_W_up, B_W_down, gate_w)
```

```python
import jax
import jax.numpy as jnp
from jax import lax
import jax.experimental.pallas as pl
import jax.experimental.pallas.tpu as pltpu

S, D, H, DH, F = 2048, 640, 32, 20, 1536
W = 24
LOG2E = 1.4426950408889634
f32, bf16, u32 = jnp.float32, jnp.bfloat16, jnp.uint32
NT = (((1,), (1,)), ((), ()))
TK = 128
NC = S // TK
SCORE_BOUND = 60.0
V_HI = 2.0 ** 40
V_LO = 2.0 ** -30


def make_kernel(tq, nxc, vr, vr0, lead, upb, tks, fb, rb, ob, wq_first, late_at):
    xc = S // nxc
    nbody = H // upb
    nvmax = max(sum(vr), sum(vr0))
    last_par = (nbody - 1) % 2

    def vcfg(v):
        nv = sum(v)
        ngroups = nv // 8
        gps = [ngroups // NC + (1 if c < ngroups % NC else 0) for c in range(NC)]
        return dict(vr=v, nv=nv, blk_row=[c * TK + 16 * b for c in range(NC) for b in range(v[c] // 16)],
                    glo=[sum(gps[:c]) for c in range(NC + 1)])

    vu = [max(a, b) for a, b in zip(vr, vr0)]
    kbo = [sum(vu[:c]) for c in range(NC + 1)]
    cfg_loop, cfg_first = vcfg(vr), vcfg(vr0)

    def kb_row(key_row):
        c, r = divmod(key_row, TK)
        return kbo[c] + r

    def kernel(x_hbm, wq_hbm, wkT_hbm, wvT_hbm, wo_hbm, wg_hbm, wu_hbm, wd_hbm, gw_hbm,
               o_ref,
               x_ref, wq_ref, wkT_ref, wvT_ref, wo_ref, wg_ref, wu_ref, wd_ref, gw_ref, sems,
               k_ref, vT_ref, wqT_ref, qT_ref, oT_ref, kb_ref, qb_ref, tok_ref, stat_ref, h_ref, *p_refs):
        step = pl.program_id(0)

        def x_copy(j):
            return pltpu.make_async_copy(x_hbm.at[pl.ds(j * xc, xc)], x_ref.at[pl.ds(j * xc, xc)], sems.at[j])

        small = [(wkT_hbm, wkT_ref), (wvT_hbm, wvT_ref), (gw_hbm, gw_ref), (wq_hbm, wq_ref)]
        late = [(wg_hbm, wg_ref), (wu_hbm, wu_ref), (wd_hbm, wd_ref), (wo_hbm, wo_ref)]

        def small_copy(j):
            return pltpu.make_async_copy(small[j][0], small[j][1], sems.at[nxc + j])

        def late_copy(j):
            return pltpu.make_async_copy(late[j][0], late[j][1], sems.at[nxc + 4 + j])

        @pl.when(step == 0)
        def _prologue():
            small_copy(0).start()
            small_copy(1).start()
            if wq_first:
                small_copy(3).start()
            for j in range(nxc):
                x_copy(j).start()
            if not wq_first:
                small_copy(3).start()
            small_copy(2).start()
            if late_at < 0:
                for j in range(4):
                    late_copy(j).start()
            small_copy(0).wait()
            small_copy(1).wait()
            r = lax.broadcasted_iota(jnp.int32, (2 * W, DH), 0)
            c = lax.broadcasted_iota(jnp.int32, (2 * W, DH), 1)
            Rk = jnp.where(r == c, 1.0, 0.0).astype(bf16)
            Rv = jnp.where(r == c + W, 1.0, 0.0).astype(bf16)
            wkvT = (jnp.dot(Rk, wkT_ref[...], preferred_element_type=f32)
                    + jnp.dot(Rv, wvT_ref[...], preferred_element_type=f32)).astype(bf16)
            if wq_first:
                small_copy(3).wait()
                wqT_ref[...] = wq_ref[...].astype(f32).T.astype(bf16)
            row = lax.broadcasted_iota(jnp.int32, (W, xc), 0)
            r = lax.broadcasted_iota(jnp.int32, (W, DH * 128), 0)
            c = lax.broadcasted_iota(jnp.int32, (W, DH * 128), 1)
            E = jnp.where(r == c // 128, 1.0, 0.0).astype(bf16)
            kmax = None
            vmax = None
            for j in range(nxc):
                x_copy(j).wait()
                if j == late_at:
                    for jj in range(4):
                        late_copy(jj).start()
                rows = pl.ds(j * xc, xc)
                kvT = lax.dot_general(wkvT, x_ref[rows, :], NT, preferred_element_type=f32)
                kvT = kvT.astype(bf16).astype(f32)
                kT, vT = kvT[0:W], kvT[W:2 * W]
                am = jnp.abs(kvT)
                kmax = am[0:W] if kmax is None else jnp.maximum(kmax, am[0:W])
                vmax = am[W:2 * W] if vmax is None else jnp.maximum(vmax, am[W:2 * W])
                vT_ref[0:W, rows] = jnp.where(row == 20, 1.0, vT)
                vT_ref[W:2 * W, rows] = jnp.where(row == 0, 1.0, pltpu.roll(vT, 4, 0))
                kk = jnp.concatenate([kT, jnp.zeros((8, xc), f32), pltpu.roll(kT, 4, 0), jnp.zeros((72, xc), f32)], axis=0)
                k4 = kk.T
                k0 = k4[:, 0:W].astype(bf16)
                k_ref[0, rows, :] = k0
                k_ref[1, rows, :] = k4[:, 32:32 + W].astype(bf16)
                if nvmax:
                    cs = [c for c in range(j * xc // TK, (j + 1) * xc // TK) if vu[c]]
                    ksel = jnp.concatenate([k0[c * TK - j * xc:c * TK - j * xc + vu[c]] for c in cs], axis=0)
                    kb_ref[pl.ds(kbo[cs[0]], ksel.shape[0]), :] = jnp.dot(ksel, E, preferred_element_type=f32)
            vmx = jnp.max(vmax)
            v_ok = jnp.logical_and(vmx <= V_HI, vmx >= V_LO)
            stat_ref[0] = jnp.where(v_ok, jnp.max(kmax) * (DH * 1.02), jnp.inf)
            if not wq_first:
                small_copy(3).wait()
                wqT_ref[...] = wq_ref[...].astype(f32).T.astype(bf16)
            small_copy(2).wait()

        row0 = pl.multiple_of(step * tq, tq)
        xb = x_ref[pl.ds(row0, tq), :]
        qT = lax.dot_general(wqT_ref[...], xb, NT, preferred_element_type=f32) * (DH ** -0.5 * LOG2E)
        qT_ref[...] = qT
        qmax = jnp.max(jnp.max(jnp.abs(qT).reshape(D // 8, 8, tq), axis=0))
        fast = qmax * stat_ref[0] <= SCORE_BOUND

        lrow = (20, 0)

        def mult(v, k):
            return v if isinstance(v, int) else pl.multiple_of(v, k)

        def store_head(base, e, o):
            if e == 0:
                oT_ref[pl.ds(base, W), :] = o
            else:
                r8 = lax.broadcasted_iota(jnp.int32, (8, tq), 0)
                oT_ref[pl.ds(base + 16, 8), :] = jnp.where(r8 < 4, oT_ref[pl.ds(base + 16, 8), :], o[0:8])
                oT_ref[pl.ds(base + 24, 16), :] = o[8:24]

        def a_slot(st, cfg, bi, par, u, c):
            e = u % 2
            key = ('A', u)
            buf = upb * par + u
            v, glo, blk_row = cfg['vr'], cfg['glo'], cfg['blk_row']
            if key not in st:
                qwin = qT_ref[pl.ds(mult(20 * upb * bi + 40 * (u // 2) + 16 * e, 8), W), :]
                st[key] = dict(qa=qwin.astype(bf16), val=None, half=None)
                if cfg['nv']:
                    for d in range(DH):
                        qb_ref[u, d] = jnp.broadcast_to(qwin[4 * e + d:4 * e + d + 1, :], (8, tq))
            a = st[key]

            def chain(f):
                a['val'] = f if a['val'] is None else jnp.maximum(a['val'], f)

            lo, n = c * TK + v[c], TK - v[c]
            s = jnp.dot(k_ref[e, pl.ds(lo, n), :], a['qa'], preferred_element_type=f32)
            p_refs[buf][pl.ds(lo // 2, n // 2), :] = pltpu.bitcast(jnp.exp2(s).astype(bf16), u32)
            chain(s[0:8])
            for g in range(glo[c], glo[c + 1]):
                krow = kb_row(blk_row[g // 2] + 8 * (g % 2))
                sv = None
                for d in range(DH):
                    kb = kb_ref[pl.ds(krow, 8), pl.ds(128 * d, 128)]
                    kbt = jnp.concatenate([kb] * (tq // 128), axis=1)
                    t = kbt * qb_ref[u, d]
                    sv = t if sv is None else sv + t
                chain(sv)
                pv = jnp.exp2(sv)
                if g % 2 == 0:
                    a['half'] = pv
                else:
                    pu = pltpu.bitcast(jnp.concatenate([a['half'], pv], axis=0).astype(bf16), u32)
                    p_refs[buf][pl.ds(blk_row[g // 2] // 2, 8), :] = pu
            if c == NC - 1:
                tok_ref[u] = a['val']
                del st[key]

        def b_slot(st, bi, par, u, c):
            e = u % 2
            buf = upb * par + u
            key = ('B', u)
            if key not in st:
                st[key] = dict(val=None)
            b = st[key]
            p = pltpu.bitcast(p_refs[buf][pl.ds(c * TK // 2, TK // 2), :], bf16)
            vt = vT_ref[W * e:W * e + W, pl.ds(c * TK, TK)]
            pv = jnp.dot(vt, p, preferred_element_type=f32)
            b['val'] = pv if b['val'] is None else b['val'] + pv
            if c == NC - 1:
                acc = b['val']
                store_head(mult(20 * upb * bi + 40 * (u // 2), 8), e, acc * (1.0 / acc[lrow[e]:lrow[e] + 1]))
                del st[key]

        def body(cfg, ia, para, ib, parb):
            st = {}
            nb = 0
            nt = upb * NC
            for t in range(nt):
                if ia is not None:
                    a_slot(st, cfg, ia, para, t // NC, t % NC)
                if ib is not None:
                    while nb < nt and nb <= t + lead:
                        b_slot(st, ib, parb, nb // NC, nb % NC)
                        nb += 1
            if ib is not None:
                while nb < nt:
                    b_slot(st, ib, parb, nb // NC, nb % NC)
                    nb += 1

        def tail():
            st = {}
            nt = upb * NC
            bq = list(range(nt))

            def b_some(n):
                for _ in range(n):
                    if bq:
                        t = bq.pop(0)
                        b_slot(st, nbody - 1, last_par, t // NC, t % NC)

            nfb = F // fb
            per = -(-nt // (2 * nfb * (tq // rb)))
            for j in range(nfb):
                cols = pl.ds(j * fb, fb)
                for r in range(tq // rb):
                    xr = x_ref[pl.ds(row0 + r * rb, rb), :]
                    gate = jnp.dot(xr, wg_ref[:, cols], preferred_element_type=f32)
                    b_some(per)
                    up = jnp.dot(xr, wu_ref[:, cols], preferred_element_type=f32)
                    b_some(per)
                    h_ref[pl.ds(r * rb, rb), cols] = (jnp.maximum(gate, 0.0) * up).astype(bf16)
            b_some(nt)
            o_all = oT_ref[...].T.astype(bf16)
            gw = gw_ref[...].astype(f32)
            for r in range(tq // ob):
                rows = pl.ds(r * ob, ob)
                a_out = jnp.dot(o_all[r * ob:(r + 1) * ob], wo_ref[...], preferred_element_type=f32)
                b_out = jnp.dot(h_ref[rows, :], wd_ref[...], preferred_element_type=f32)
                xf = x_ref[pl.ds(row0 + r * ob, ob), :].astype(f32)
                la = xf[:, 0:128] * gw[0:1, :]
                for j in range(1, D // 128):
                    la = la + xf[:, 128 * j:128 * (j + 1)] * gw[j:j + 1, :]
                g = jax.nn.sigmoid(jnp.sum(la, axis=-1, keepdims=True))
                o_ref[rows, :] = (g * a_out + (1.0 - g) * b_out).astype(o_ref.dtype)

        body(cfg_first, 0, 0, None, None)

        @pl.when(fast)
        def _fast():
            def loop_body(i, carry):
                @pl.when(i % 2 == 0)
                def _():
                    body(cfg_loop, i + 1, 1, i, 0)

                @pl.when(i % 2 == 1)
                def _():
                    body(cfg_loop, i + 1, 0, i, 1)
                return carry

            lax.fori_loop(0, nbody - 1, loop_body, 0)

        @pl.when(jnp.logical_not(fast))
        def _slow():
            def q_of(pi, e):
                return qT_ref[pl.ds(mult(40 * pi + 16 * e, 8), W), :].astype(bf16)

            def scores(e, qa, j):
                r0 = pl.multiple_of(j * tks, tks)
                return r0, jnp.dot(k_ref[e, pl.ds(r0, tks), :], qa, preferred_element_type=f32)

            def pair_body(pi, carry):
                for e in range(2):
                    qa = q_of(pi, e)

                    def chunk(j, mc):
                        m, acc = mc
                        r0, s = scores(e, qa, j)
                        m_new = jnp.maximum(m, jnp.max(s, axis=0, keepdims=True))
                        p = jnp.exp2(s - m_new).astype(bf16)
                        pv = jnp.dot(vT_ref[W * e:W * e + W, pl.ds(r0, tks)], p, preferred_element_type=f32)
                        return m_new, acc * jnp.exp2(m - m_new) + pv

                    m0 = jnp.full((1, tq), -jnp.inf, f32)
                    _, acc = lax.fori_loop(0, S // tks, chunk, (m0, jnp.zeros((W, tq), f32)))
                    store_head(pl.multiple_of(40 * pi, 8), e, acc * (1.0 / acc[lrow[e]:lrow[e] + 1]))
                return carry

            lax.fori_loop(0, (H - upb) // 2, pair_body, 0)
            for u in range(upb):
                e = u % 2
                qa = q_of((H - upb) // 2 + u // 2, e)
                buf = upb * last_par + u

                def row_max(j, m):
                    return jnp.maximum(m, jnp.max(scores(e, qa, j)[1], axis=0, keepdims=True))

                m = lax.fori_loop(0, S // tks, row_max, jnp.full((1, tq), -jnp.inf, f32))

                def write_p(j, carry):
                    r0, s = scores(e, qa, j)
                    p = pltpu.bitcast(jnp.exp2(s - m).astype(bf16), u32)
                    p_refs[buf][pl.ds(pl.multiple_of(j * (tks // 2), tks // 2), tks // 2), :] = p
                    return carry

                lax.fori_loop(0, S // tks, write_p, 0)

        @pl.when(step == 0)
        def _wait_late():
            for j in range(4):
                late_copy(j).wait()

        tail()
    return kernel


def build(tq=512, nxc=4, vr=None, vr0=None, lead=-1, upb=4, tks=256, fb=512, rb=128, ob=256, wq_first=1, late_at=-1):
    if vr is None:
        vr = [16, 0] * 8
    if vr0 is None:
        vr0 = [16] * 16

    def run(A_x, A_wq, A_wk, A_wv, A_wo, B_x, B_W_gate, B_W_up, B_W_down, gate_w):
        x = A_x.reshape(S, D)
        gw = gate_w.reshape(D // 128, 128)
        hbm = pl.BlockSpec(memory_space=pl.ANY)
        nvu = sum(max(a, b) for a, b in zip(vr, vr0))
        out = pl.pallas_call(
            make_kernel(tq, nxc, tuple(vr), tuple(vr0), lead, upb, tks, fb, rb, ob, wq_first, late_at),
            grid=(S // tq,),
            in_specs=[hbm] * 9,
            out_specs=pl.BlockSpec((tq, D), lambda i: (i, 0)),
            out_shape=jax.ShapeDtypeStruct((S, D), bf16),
            scratch_shapes=[
                pltpu.VMEM((S, D), bf16),
                pltpu.VMEM((D, D), bf16),
                pltpu.VMEM((DH, D), bf16),
                pltpu.VMEM((DH, D), bf16),
                pltpu.VMEM((D, D), bf16),
                pltpu.VMEM((D, F), bf16),
                pltpu.VMEM((D, F), bf16),
                pltpu.VMEM((F, D), bf16),
                pltpu.VMEM((D // 128, 128), bf16),
                pltpu.SemaphoreType.DMA((nxc + 8,)),
                pltpu.VMEM((2, S, W), bf16),
                pltpu.VMEM((2 * W, S), f32),
                pltpu.VMEM((D, D), bf16),
                pltpu.VMEM((D, tq), f32),
                pltpu.VMEM((D, tq), f32),
                pltpu.VMEM((max(nvu, 8), DH * 128), f32),
                pltpu.VMEM((upb, DH, 8, tq), f32),
                pltpu.VMEM((upb, 8, tq), f32),
                pltpu.SMEM((1,), f32),
                pltpu.VMEM((tq, F), bf16),
            ] + [pltpu.VMEM((S // 2, tq), u32)] * (2 * upb),
            compiler_params=pltpu.CompilerParams(
                dimension_semantics=("arbitrary",), vmem_limit_bytes=120 * 1024 * 1024),
        )(x, A_wq, A_wk.T, A_wv.T, A_wo, B_W_gate, B_W_up, B_W_down, gw)
        return out.reshape(1, S, D)
    return jax.jit(run)


_RUN = build(wq_first=0)


@jax.jit
def pallas_gated_mix__grouped_kv_mqa__glu_gated_reglu__prompt_kernel(
    A_x: jax.Array,
    A_wq: jax.Array,
    A_wk: jax.Array,
    A_wv: jax.Array,
    A_wo: jax.Array,
    B_x: jax.Array,
    B_W_gate: jax.Array,
    B_W_up: jax.Array,
    B_W_down: jax.Array,
    gate_w: jax.Array,
):
    return _RUN(A_x, A_wq, A_wk, A_wv, A_wo, B_x, B_W_gate, B_W_up, B_W_down, gate_w)
```

```python
import jax
import jax.numpy as jnp
from jax import lax
import jax.experimental.pallas as pl
import jax.experimental.pallas.tpu as pltpu

S, D, H, DH, F = 2048, 640, 32, 20, 1536
W = 24
LOG2E = 1.4426950408889634
f32, bf16, u32 = jnp.float32, jnp.bfloat16, jnp.uint32
NT = (((1,), (1,)), ((), ()))
TK = 128
NC = S // TK
SCORE_BOUND = 60.0
V_HI = 2.0 ** 40
V_LO = 2.0 ** -30


def make_kernel(tq, nxc, vr, vr0, lead, upb, tks, fb, rb, ob, wq_first, late_at):
    xc = S // nxc
    nbody = H // upb
    nvmax = max(sum(vr), sum(vr0))
    last_par = (nbody - 1) % 2

    def vcfg(v):
        nv = sum(v)
        ngroups = nv // 8
        gps = [ngroups // NC + (1 if c < ngroups % NC else 0) for c in range(NC)]
        return dict(vr=v, nv=nv, blk_row=[c * TK + 16 * b for c in range(NC) for b in range(v[c] // 16)],
                    glo=[sum(gps[:c]) for c in range(NC + 1)])

    vu = [max(a, b) for a, b in zip(vr, vr0)]
    kbo = [sum(vu[:c]) for c in range(NC + 1)]
    cfg_loop, cfg_first = vcfg(vr), vcfg(vr0)

    def kb_row(key_row):
        c, r = divmod(key_row, TK)
        return kbo[c] + r

    def kernel(x_hbm, wq_hbm, wkT_hbm, wvT_hbm, wo_hbm, wg_hbm, wu_hbm, wd_hbm, gw_hbm,
               o_hbm,
               x_ref, wq_ref, wkT_ref, wvT_ref, wo_ref, wg_ref, wu_ref, wd_ref, gw_ref, sems,
               k_ref, vT_ref, wqT_ref, qT_ref, oT_ref, kb_ref, qb_ref, tok_ref, stat_ref, h_ref, ob_ref, osems, *p_refs):
        step = pl.program_id(0)

        def x_copy(j):
            return pltpu.make_async_copy(x_hbm.at[pl.ds(j * xc, xc)], x_ref.at[pl.ds(j * xc, xc)], sems.at[j])

        small = [(wkT_hbm, wkT_ref), (wvT_hbm, wvT_ref), (gw_hbm, gw_ref), (wq_hbm, wq_ref)]
        late = [(wg_hbm, wg_ref), (wu_hbm, wu_ref), (wd_hbm, wd_ref), (wo_hbm, wo_ref)]

        def small_copy(j):
            return pltpu.make_async_copy(small[j][0], small[j][1], sems.at[nxc + j])

        def late_copy(j):
            return pltpu.make_async_copy(late[j][0], late[j][1], sems.at[nxc + 4 + j])

        def out_copy(s, r):
            return pltpu.make_async_copy(ob_ref.at[pl.ds(r * ob, ob)],
                                         o_hbm.at[pl.ds(pl.multiple_of(s * tq + r * ob, ob), ob)], osems.at[r])

        @pl.when(step == 0)
        def _prologue():
            small_copy(0).start()
            small_copy(1).start()
            if wq_first:
                small_copy(3).start()
            for j in range(nxc):
                x_copy(j).start()
            if not wq_first:
                small_copy(3).start()
            small_copy(2).start()
            if late_at < 0:
                for j in range(4):
                    late_copy(j).start()
            small_copy(0).wait()
            small_copy(1).wait()
            r = lax.broadcasted_iota(jnp.int32, (2 * W, DH), 0)
            c = lax.broadcasted_iota(jnp.int32, (2 * W, DH), 1)
            Rk = jnp.where(r == c, 1.0, 0.0).astype(bf16)
            Rv = jnp.where(r == c + W, 1.0, 0.0).astype(bf16)
            wkvT = (jnp.dot(Rk, wkT_ref[...], preferred_element_type=f32)
                    + jnp.dot(Rv, wvT_ref[...], preferred_element_type=f32)).astype(bf16)
            if wq_first:
                small_copy(3).wait()
                wqT_ref[...] = wq_ref[...].astype(f32).T.astype(bf16)
            row = lax.broadcasted_iota(jnp.int32, (W, xc), 0)
            r = lax.broadcasted_iota(jnp.int32, (W, DH * 128), 0)
            c = lax.broadcasted_iota(jnp.int32, (W, DH * 128), 1)
            E = jnp.where(r == c // 128, 1.0, 0.0).astype(bf16)
            kmax = None
            vmax = None
            for j in range(nxc):
                x_copy(j).wait()
                if j == late_at:
                    for jj in range(4):
                        late_copy(jj).start()
                rows = pl.ds(j * xc, xc)
                kvT = lax.dot_general(wkvT, x_ref[rows, :], NT, preferred_element_type=f32)
                kvT = kvT.astype(bf16).astype(f32)
                kT, vT = kvT[0:W], kvT[W:2 * W]
                am = jnp.abs(kvT)
                kmax = am[0:W] if kmax is None else jnp.maximum(kmax, am[0:W])
                vmax = am[W:2 * W] if vmax is None else jnp.maximum(vmax, am[W:2 * W])
                vT_ref[0:W, rows] = jnp.where(row == 20, 1.0, vT)
                vT_ref[W:2 * W, rows] = jnp.where(row == 0, 1.0, pltpu.roll(vT, 4, 0))
                kk = jnp.concatenate([kT, jnp.zeros((8, xc), f32), pltpu.roll(kT, 4, 0), jnp.zeros((72, xc), f32)], axis=0)
                k4 = kk.T
                k0 = k4[:, 0:W].astype(bf16)
                k_ref[0, rows, :] = k0
                k_ref[1, rows, :] = k4[:, 32:32 + W].astype(bf16)
                if nvmax:
                    cs = [c for c in range(j * xc // TK, (j + 1) * xc // TK) if vu[c]]
                    ksel = jnp.concatenate([k0[c * TK - j * xc:c * TK - j * xc + vu[c]] for c in cs], axis=0)
                    kb_ref[pl.ds(kbo[cs[0]], ksel.shape[0]), :] = jnp.dot(ksel, E, preferred_element_type=f32)
            vmx = jnp.max(vmax)
            v_ok = jnp.logical_and(vmx <= V_HI, vmx >= V_LO)
            stat_ref[0] = jnp.where(v_ok, jnp.max(kmax) * (DH * 1.02), jnp.inf)
            if not wq_first:
                small_copy(3).wait()
                wqT_ref[...] = wq_ref[...].astype(f32).T.astype(bf16)
            small_copy(2).wait()

        row0 = pl.multiple_of(step * tq, tq)
        xb = x_ref[pl.ds(row0, tq), :]
        qT = lax.dot_general(wqT_ref[...], xb, NT, preferred_element_type=f32) * (DH ** -0.5 * LOG2E)
        qT_ref[...] = qT
        qmax = jnp.max(jnp.max(jnp.abs(qT).reshape(D // 8, 8, tq), axis=0))
        fast = qmax * stat_ref[0] <= SCORE_BOUND

        lrow = (20, 0)

        def mult(v, k):
            return v if isinstance(v, int) else pl.multiple_of(v, k)

        def store_head(base, e, o):
            if e == 0:
                oT_ref[pl.ds(base, W), :] = o
            else:
                r8 = lax.broadcasted_iota(jnp.int32, (8, tq), 0)
                oT_ref[pl.ds(base + 16, 8), :] = jnp.where(r8 < 4, oT_ref[pl.ds(base + 16, 8), :], o[0:8])
                oT_ref[pl.ds(base + 24, 16), :] = o[8:24]

        def a_slot(st, cfg, bi, par, u, c):
            e = u % 2
            key = ('A', u)
            buf = upb * par + u
            v, glo, blk_row = cfg['vr'], cfg['glo'], cfg['blk_row']
            if key not in st:
                qwin = qT_ref[pl.ds(mult(20 * upb * bi + 40 * (u // 2) + 16 * e, 8), W), :]
                st[key] = dict(qa=qwin.astype(bf16), val=None, half=None)
                if cfg['nv']:
                    for d in range(DH):
                        qb_ref[u, d] = jnp.broadcast_to(qwin[4 * e + d:4 * e + d + 1, :], (8, tq))
            a = st[key]

            def chain(f):
                a['val'] = f if a['val'] is None else jnp.maximum(a['val'], f)

            lo, n = c * TK + v[c], TK - v[c]
            s = jnp.dot(k_ref[e, pl.ds(lo, n), :], a['qa'], preferred_element_type=f32)
            p_refs[buf][pl.ds(lo // 2, n // 2), :] = pltpu.bitcast(jnp.exp2(s).astype(bf16), u32)
            chain(s[0:8])
            for g in range(glo[c], glo[c + 1]):
                krow = kb_row(blk_row[g // 2] + 8 * (g % 2))
                sv = None
                for d in range(DH):
                    kb = kb_ref[pl.ds(krow, 8), pl.ds(128 * d, 128)]
                    kbt = jnp.concatenate([kb] * (tq // 128), axis=1)
                    t = kbt * qb_ref[u, d]
                    sv = t if sv is None else sv + t
                chain(sv)
                pv = jnp.exp2(sv)
                if g % 2 == 0:
                    a['half'] = pv
                else:
                    pu = pltpu.bitcast(jnp.concatenate([a['half'], pv], axis=0).astype(bf16), u32)
                    p_refs[buf][pl.ds(blk_row[g // 2] // 2, 8), :] = pu
            if c == NC - 1:
                tok_ref[u] = a['val']
                del st[key]

        def b_slot(st, bi, par, u, c):
            e = u % 2
            buf = upb * par + u
            key = ('B', u)
            if key not in st:
                st[key] = dict(val=None)
            b = st[key]
            p = pltpu.bitcast(p_refs[buf][pl.ds(c * TK // 2, TK // 2), :], bf16)
            vt = vT_ref[W * e:W * e + W, pl.ds(c * TK, TK)]
            pv = jnp.dot(vt, p, preferred_element_type=f32)
            b['val'] = pv if b['val'] is None else b['val'] + pv
            if c == NC - 1:
                acc = b['val']
                store_head(mult(20 * upb * bi + 40 * (u // 2), 8), e, acc * (1.0 / acc[lrow[e]:lrow[e] + 1]))
                del st[key]

        def body(cfg, ia, para, ib, parb):
            st = {}
            nb = 0
            nt = upb * NC
            for t in range(nt):
                if ia is not None:
                    a_slot(st, cfg, ia, para, t // NC, t % NC)
                if ib is not None:
                    while nb < nt and nb <= t + lead:
                        b_slot(st, ib, parb, nb // NC, nb % NC)
                        nb += 1
            if ib is not None:
                while nb < nt:
                    b_slot(st, ib, parb, nb // NC, nb % NC)
                    nb += 1

        def tail():
            st = {}
            nt = upb * NC
            bq = list(range(nt))

            def b_some(n):
                for _ in range(n):
                    if bq:
                        t = bq.pop(0)
                        b_slot(st, nbody - 1, last_par, t // NC, t % NC)

            nfb = F // fb
            per = -(-nt // (2 * nfb * (tq // rb)))
            for j in range(nfb):
                cols = pl.ds(j * fb, fb)
                for r in range(tq // rb):
                    xr = x_ref[pl.ds(row0 + r * rb, rb), :]
                    gate = jnp.dot(xr, wg_ref[:, cols], preferred_element_type=f32)
                    b_some(per)
                    up = jnp.dot(xr, wu_ref[:, cols], preferred_element_type=f32)
                    b_some(per)
                    h_ref[pl.ds(r * rb, rb), cols] = (jnp.maximum(gate, 0.0) * up).astype(bf16)
            b_some(nt)
            o_all = oT_ref[...].T.astype(bf16)
            gw = gw_ref[...].astype(f32)
            for r in range(tq // ob):
                rows = pl.ds(r * ob, ob)
                a_out = jnp.dot(o_all[r * ob:(r + 1) * ob], wo_ref[...], preferred_element_type=f32)
                b_out = jnp.dot(h_ref[rows, :], wd_ref[...], preferred_element_type=f32)
                xf = x_ref[pl.ds(row0 + r * ob, ob), :].astype(f32)
                la = xf[:, 0:128] * gw[0:1, :]
                for j in range(1, D // 128):
                    la = la + xf[:, 128 * j:128 * (j + 1)] * gw[j:j + 1, :]
                g = jax.nn.sigmoid(jnp.sum(la, axis=-1, keepdims=True))
                ob_ref[rows, :] = (g * a_out + (1.0 - g) * b_out).astype(bf16)
                out_copy(step, r).start()

        body(cfg_first, 0, 0, None, None)

        @pl.when(fast)
        def _fast():
            def loop_body(i, carry):
                @pl.when(i % 2 == 0)
                def _():
                    body(cfg_loop, i + 1, 1, i, 0)

                @pl.when(i % 2 == 1)
                def _():
                    body(cfg_loop, i + 1, 0, i, 1)
                return carry

            lax.fori_loop(0, nbody - 1, loop_body, 0)

        @pl.when(jnp.logical_not(fast))
        def _slow():
            def q_of(pi, e):
                return qT_ref[pl.ds(mult(40 * pi + 16 * e, 8), W), :].astype(bf16)

            def scores(e, qa, j):
                r0 = pl.multiple_of(j * tks, tks)
                return r0, jnp.dot(k_ref[e, pl.ds(r0, tks), :], qa, preferred_element_type=f32)

            def pair_body(pi, carry):
                for e in range(2):
                    qa = q_of(pi, e)

                    def chunk(j, mc):
                        m, acc = mc
                        r0, s = scores(e, qa, j)
                        m_new = jnp.maximum(m, jnp.max(s, axis=0, keepdims=True))
                        p = jnp.exp2(s - m_new).astype(bf16)
                        pv = jnp.dot(vT_ref[W * e:W * e + W, pl.ds(r0, tks)], p, preferred_element_type=f32)
                        return m_new, acc * jnp.exp2(m - m_new) + pv

                    m0 = jnp.full((1, tq), -jnp.inf, f32)
                    _, acc = lax.fori_loop(0, S // tks, chunk, (m0, jnp.zeros((W, tq), f32)))
                    store_head(pl.multiple_of(40 * pi, 8), e, acc * (1.0 / acc[lrow[e]:lrow[e] + 1]))
                return carry

            lax.fori_loop(0, (H - upb) // 2, pair_body, 0)
            for u in range(upb):
                e = u % 2
                qa = q_of((H - upb) // 2 + u // 2, e)
                buf = upb * last_par + u

                def row_max(j, m):
                    return jnp.maximum(m, jnp.max(scores(e, qa, j)[1], axis=0, keepdims=True))

                m = lax.fori_loop(0, S // tks, row_max, jnp.full((1, tq), -jnp.inf, f32))

                def write_p(j, carry):
                    r0, s = scores(e, qa, j)
                    p = pltpu.bitcast(jnp.exp2(s - m).astype(bf16), u32)
                    p_refs[buf][pl.ds(pl.multiple_of(j * (tks // 2), tks // 2), tks // 2), :] = p
                    return carry

                lax.fori_loop(0, S // tks, write_p, 0)

        @pl.when(step == 0)
        def _wait_late():
            for j in range(4):
                late_copy(j).wait()

        @pl.when(step > 0)
        def _wait_prev_out():
            for r in range(tq // ob):
                out_copy(step - 1, r).wait()

        tail()

        @pl.when(step == S // tq - 1)
        def _wait_out():
            for r in range(tq // ob):
                out_copy(step, r).wait()
    return kernel


def build(tq=512, nxc=4, vr=None, vr0=None, lead=-1, upb=4, tks=256, fb=512, rb=128, ob=256, wq_first=0, late_at=-1):
    if vr is None:
        vr = [16, 0] * 8
    if vr0 is None:
        vr0 = [16] * 16

    def run(A_x, A_wq, A_wk, A_wv, A_wo, B_x, B_W_gate, B_W_up, B_W_down, gate_w):
        x = A_x.reshape(S, D)
        gw = gate_w.reshape(D // 128, 128)
        hbm = pl.BlockSpec(memory_space=pl.ANY)
        nvu = sum(max(a, b) for a, b in zip(vr, vr0))
        out = pl.pallas_call(
            make_kernel(tq, nxc, tuple(vr), tuple(vr0), lead, upb, tks, fb, rb, ob, wq_first, late_at),
            grid=(S // tq,),
            in_specs=[hbm] * 9,
            out_specs=hbm,
            out_shape=jax.ShapeDtypeStruct((S, D), bf16),
            scratch_shapes=[
                pltpu.VMEM((S, D), bf16),
                pltpu.VMEM((D, D), bf16),
                pltpu.VMEM((DH, D), bf16),
                pltpu.VMEM((DH, D), bf16),
                pltpu.VMEM((D, D), bf16),
                pltpu.VMEM((D, F), bf16),
                pltpu.VMEM((D, F), bf16),
                pltpu.VMEM((F, D), bf16),
                pltpu.VMEM((D // 128, 128), bf16),
                pltpu.SemaphoreType.DMA((nxc + 8,)),
                pltpu.VMEM((2, S, W), bf16),
                pltpu.VMEM((2 * W, S), f32),
                pltpu.VMEM((D, D), bf16),
                pltpu.VMEM((D, tq), f32),
                pltpu.VMEM((D, tq), f32),
                pltpu.VMEM((max(nvu, 8), DH * 128), f32),
                pltpu.VMEM((upb, DH, 8, tq), f32),
                pltpu.VMEM((upb, 8, tq), f32),
                pltpu.SMEM((1,), f32),
                pltpu.VMEM((tq, F), bf16),
                pltpu.VMEM((tq, D), bf16),
                pltpu.SemaphoreType.DMA((tq // ob,)),
            ] + [pltpu.VMEM((S // 2, tq), u32)] * (2 * upb),
            compiler_params=pltpu.CompilerParams(
                dimension_semantics=("arbitrary",), vmem_limit_bytes=120 * 1024 * 1024),
        )(x, A_wq, A_wk.T, A_wv.T, A_wo, B_W_gate, B_W_up, B_W_down, gw)
        return out.reshape(1, S, D)
    return jax.jit(run)


_RUN = build(ob=128)


@jax.jit
def pallas_gated_mix__grouped_kv_mqa__glu_gated_reglu__prompt_kernel(
    A_x: jax.Array,
    A_wq: jax.Array,
    A_wk: jax.Array,
    A_wv: jax.Array,
    A_wo: jax.Array,
    B_x: jax.Array,
    B_W_gate: jax.Array,
    B_W_up: jax.Array,
    B_W_down: jax.Array,
    gate_w: jax.Array,
):
    return _RUN(A_x, A_wq, A_wk, A_wv, A_wo, B_x, B_W_gate, B_W_up, B_W_down, gate_w)
```

```python
import jax
import jax.numpy as jnp
from jax import lax
import jax.experimental.pallas as pl
import jax.experimental.pallas.tpu as pltpu

S, D, H, DH, F = 2048, 640, 32, 20, 1536
W = 24
LOG2E = 1.4426950408889634
f32, bf16, u32 = jnp.float32, jnp.bfloat16, jnp.uint32
NT = (((1,), (1,)), ((), ()))

TQ = 512
TK = 128
NC = S // TK
NXC = 4
XC = S // NXC
UPB = 4
NGRP = H // UPB
LAST_PAR = (NGRP - 1) % 2
LEAD = -1
TKS = 256
FB, RB, OB = 512, 128, 128
VR_LOOP = (16, 0) * 8
VR_FIRST = (16,) * 16

SCORE_BOUND = 60.0
V_HI = 2.0 ** 40
V_LO = 2.0 ** -30


def _vcfg(v):
    ngroups = sum(v) // 8
    gps = [ngroups // NC + (1 if c < ngroups % NC else 0) for c in range(NC)]
    return dict(vr=v, blk_row=[c * TK + 16 * b for c in range(NC) for b in range(v[c] // 16)],
                glo=[sum(gps[:c]) for c in range(NC + 1)])


VU = [max(a, b) for a, b in zip(VR_LOOP, VR_FIRST)]
KBO = [sum(VU[:c]) for c in range(NC + 1)]
CFG_LOOP, CFG_FIRST = _vcfg(VR_LOOP), _vcfg(VR_FIRST)


def _kb_row(key_row):
    c, r = divmod(key_row, TK)
    return KBO[c] + r


def _mult(v, k):
    return v if isinstance(v, int) else pl.multiple_of(v, k)


def _kernel(x_hbm, wq_hbm, wkT_hbm, wvT_hbm, wo_hbm, wg_hbm, wu_hbm, wd_hbm, gw_hbm,
            o_hbm,
            x_ref, wq_ref, wkT_ref, wvT_ref, wo_ref, wg_ref, wu_ref, wd_ref, gw_ref, sems,
            k_ref, vT_ref, wqT_ref, qT_ref, oT_ref, kb_ref, qb_ref, tok_ref, stat_ref, h_ref, ob_ref, osems,
            *p_refs):
    step = pl.program_id(0)
    tq = TQ

    def x_copy(j):
        return pltpu.make_async_copy(x_hbm.at[pl.ds(j * XC, XC)], x_ref.at[pl.ds(j * XC, XC)], sems.at[j])

    small = [(wkT_hbm, wkT_ref), (wvT_hbm, wvT_ref), (gw_hbm, gw_ref), (wq_hbm, wq_ref)]
    late = [(wg_hbm, wg_ref), (wu_hbm, wu_ref), (wd_hbm, wd_ref), (wo_hbm, wo_ref)]

    def small_copy(j):
        return pltpu.make_async_copy(small[j][0], small[j][1], sems.at[NXC + j])

    def late_copy(j):
        return pltpu.make_async_copy(late[j][0], late[j][1], sems.at[NXC + 4 + j])

    def out_copy(s, r):
        return pltpu.make_async_copy(ob_ref.at[pl.ds(r * OB, OB)],
                                     o_hbm.at[pl.ds(pl.multiple_of(s * tq + r * OB, OB), OB)], osems.at[r])

    @pl.when(step == 0)
    def _prologue():
        small_copy(0).start()
        small_copy(1).start()
        for j in range(NXC):
            x_copy(j).start()
        small_copy(3).start()
        small_copy(2).start()
        for j in range(4):
            late_copy(j).start()
        small_copy(0).wait()
        small_copy(1).wait()
        r = lax.broadcasted_iota(jnp.int32, (2 * W, DH), 0)
        c = lax.broadcasted_iota(jnp.int32, (2 * W, DH), 1)
        Rk = jnp.where(r == c, 1.0, 0.0).astype(bf16)
        Rv = jnp.where(r == c + W, 1.0, 0.0).astype(bf16)
        wkvT = (jnp.dot(Rk, wkT_ref[...], preferred_element_type=f32)
                + jnp.dot(Rv, wvT_ref[...], preferred_element_type=f32)).astype(bf16)
        row = lax.broadcasted_iota(jnp.int32, (W, XC), 0)
        r = lax.broadcasted_iota(jnp.int32, (W, DH * 128), 0)
        c = lax.broadcasted_iota(jnp.int32, (W, DH * 128), 1)
        E = jnp.where(r == c // 128, 1.0, 0.0).astype(bf16)
        kmax = None
        vmax = None
        for j in range(NXC):
            x_copy(j).wait()
            rows = pl.ds(j * XC, XC)
            kvT = lax.dot_general(wkvT, x_ref[rows, :], NT, preferred_element_type=f32)
            kvT = kvT.astype(bf16).astype(f32)
            kT, vT = kvT[0:W], kvT[W:2 * W]
            am = jnp.abs(kvT)
            kmax = am[0:W] if kmax is None else jnp.maximum(kmax, am[0:W])
            vmax = am[W:2 * W] if vmax is None else jnp.maximum(vmax, am[W:2 * W])
            vT_ref[0:W, rows] = jnp.where(row == 20, 1.0, vT)
            vT_ref[W:2 * W, rows] = jnp.where(row == 0, 1.0, pltpu.roll(vT, 4, 0))
            kk = jnp.concatenate([kT, jnp.zeros((8, XC), f32), pltpu.roll(kT, 4, 0), jnp.zeros((72, XC), f32)],
                                 axis=0)
            k4 = kk.T
            k0 = k4[:, 0:W].astype(bf16)
            k_ref[0, rows, :] = k0
            k_ref[1, rows, :] = k4[:, 32:32 + W].astype(bf16)
            cs = [c for c in range(j * XC // TK, (j + 1) * XC // TK) if VU[c]]
            ksel = jnp.concatenate([k0[c * TK - j * XC:c * TK - j * XC + VU[c]] for c in cs], axis=0)
            kb_ref[pl.ds(KBO[cs[0]], ksel.shape[0]), :] = jnp.dot(ksel, E, preferred_element_type=f32)
        vmx = jnp.max(vmax)
        v_ok = jnp.logical_and(vmx <= V_HI, vmx >= V_LO)
        stat_ref[0] = jnp.where(v_ok, jnp.max(kmax) * (DH * 1.02), jnp.inf)
        small_copy(3).wait()
        wqT_ref[...] = wq_ref[...].astype(f32).T.astype(bf16)
        small_copy(2).wait()

    row0 = pl.multiple_of(step * tq, tq)
    xb = x_ref[pl.ds(row0, tq), :]
    qT = lax.dot_general(wqT_ref[...], xb, NT, preferred_element_type=f32) * (DH ** -0.5 * LOG2E)
    qT_ref[...] = qT
    qmax = jnp.max(jnp.max(jnp.abs(qT).reshape(D // 8, 8, tq), axis=0))
    fast = qmax * stat_ref[0] <= SCORE_BOUND

    lrow = (20, 0)

    def store_head(base, e, o):
        if e == 0:
            oT_ref[pl.ds(base, W), :] = o
        else:
            r8 = lax.broadcasted_iota(jnp.int32, (8, tq), 0)
            oT_ref[pl.ds(base + 16, 8), :] = jnp.where(r8 < 4, oT_ref[pl.ds(base + 16, 8), :], o[0:8])
            oT_ref[pl.ds(base + 24, 16), :] = o[8:24]

    def a_slot(st, cfg, bi, par, u, c):
        e = u % 2
        key = ('A', u)
        buf = UPB * par + u
        v, glo, blk_row = cfg['vr'], cfg['glo'], cfg['blk_row']
        if key not in st:
            qwin = qT_ref[pl.ds(_mult(20 * UPB * bi + 40 * (u // 2) + 16 * e, 8), W), :]
            st[key] = dict(qa=qwin.astype(bf16), val=None, half=None)
            for d in range(DH):
                qb_ref[u, d] = jnp.broadcast_to(qwin[4 * e + d:4 * e + d + 1, :], (8, tq))
        a = st[key]

        def chain(f):
            a['val'] = f if a['val'] is None else jnp.maximum(a['val'], f)

        lo, n = c * TK + v[c], TK - v[c]
        s = jnp.dot(k_ref[e, pl.ds(lo, n), :], a['qa'], preferred_element_type=f32)
        p_refs[buf][pl.ds(lo // 2, n // 2), :] = pltpu.bitcast(jnp.exp2(s).astype(bf16), u32)
        chain(s[0:8])
        for g in range(glo[c], glo[c + 1]):
            krow = _kb_row(blk_row[g // 2] + 8 * (g % 2))
            sv = None
            for d in range(DH):
                kb = kb_ref[pl.ds(krow, 8), pl.ds(128 * d, 128)]
                kbt = jnp.concatenate([kb] * (tq // 128), axis=1)
                t = kbt * qb_ref[u, d]
                sv = t if sv is None else sv + t
            chain(sv)
            pv = jnp.exp2(sv)
            if g % 2 == 0:
                a['half'] = pv
            else:
                pu = pltpu.bitcast(jnp.concatenate([a['half'], pv], axis=0).astype(bf16), u32)
                p_refs[buf][pl.ds(blk_row[g // 2] // 2, 8), :] = pu
        if c == NC - 1:
            tok_ref[u] = a['val']
            del st[key]

    def b_slot(st, bi, par, u, c):
        e = u % 2
        buf = UPB * par + u
        key = ('B', u)
        if key not in st:
            st[key] = dict(val=None)
        b = st[key]
        p = pltpu.bitcast(p_refs[buf][pl.ds(c * TK // 2, TK // 2), :], bf16)
        vt = vT_ref[W * e:W * e + W, pl.ds(c * TK, TK)]
        pv = jnp.dot(vt, p, preferred_element_type=f32)
        b['val'] = pv if b['val'] is None else b['val'] + pv
        if c == NC - 1:
            acc = b['val']
            store_head(_mult(20 * UPB * bi + 40 * (u // 2), 8), e, acc * (1.0 / acc[lrow[e]:lrow[e] + 1]))
            del st[key]

    def body(cfg, ia, para, ib, parb):
        st = {}
        nb = 0
        nt = UPB * NC
        for t in range(nt):
            if ia is not None:
                a_slot(st, cfg, ia, para, t // NC, t % NC)
            if ib is not None:
                while nb < nt and nb <= t + LEAD:
                    b_slot(st, ib, parb, nb // NC, nb % NC)
                    nb += 1
        if ib is not None:
            while nb < nt:
                b_slot(st, ib, parb, nb // NC, nb % NC)
                nb += 1

    def tail():
        st = {}
        nt = UPB * NC
        bq = list(range(nt))

        def b_some(n):
            for _ in range(n):
                if bq:
                    t = bq.pop(0)
                    b_slot(st, NGRP - 1, LAST_PAR, t // NC, t % NC)

        nfb = F // FB
        per = -(-nt // (2 * nfb * (tq // RB)))
        for j in range(nfb):
            cols = pl.ds(j * FB, FB)
            for r in range(tq // RB):
                xr = x_ref[pl.ds(row0 + r * RB, RB), :]
                gate = jnp.dot(xr, wg_ref[:, cols], preferred_element_type=f32)
                b_some(per)
                up = jnp.dot(xr, wu_ref[:, cols], preferred_element_type=f32)
                b_some(per)
                h_ref[pl.ds(r * RB, RB), cols] = (jnp.maximum(gate, 0.0) * up).astype(bf16)
        b_some(nt)
        o_all = oT_ref[...].T.astype(bf16)
        gw = gw_ref[...].astype(f32)
        for r in range(tq // OB):
            rows = pl.ds(r * OB, OB)
            a_out = jnp.dot(o_all[r * OB:(r + 1) * OB], wo_ref[...], preferred_element_type=f32)
            b_out = jnp.dot(h_ref[rows, :], wd_ref[...], preferred_element_type=f32)
            xf = x_ref[pl.ds(row0 + r * OB, OB), :].astype(f32)
            la = xf[:, 0:128] * gw[0:1, :]
            for j in range(1, D // 128):
                la = la + xf[:, 128 * j:128 * (j + 1)] * gw[j:j + 1, :]
            g = jax.nn.sigmoid(jnp.sum(la, axis=-1, keepdims=True))
            ob_ref[rows, :] = (g * a_out + (1.0 - g) * b_out).astype(bf16)
            out_copy(step, r).start()

    body(CFG_FIRST, 0, 0, None, None)

    @pl.when(fast)
    def _fast():
        def loop_body(i, carry):
            @pl.when(i % 2 == 0)
            def _():
                body(CFG_LOOP, i + 1, 1, i, 0)

            @pl.when(i % 2 == 1)
            def _():
                body(CFG_LOOP, i + 1, 0, i, 1)
            return carry

        lax.fori_loop(0, NGRP - 1, loop_body, 0)

    @pl.when(jnp.logical_not(fast))
    def _slow():
        def q_of(pi, e):
            return qT_ref[pl.ds(_mult(40 * pi + 16 * e, 8), W), :].astype(bf16)

        def scores(e, qa, j):
            r0 = pl.multiple_of(j * TKS, TKS)
            return r0, jnp.dot(k_ref[e, pl.ds(r0, TKS), :], qa, preferred_element_type=f32)

        def pair_body(pi, carry):
            for e in range(2):
                qa = q_of(pi, e)

                def chunk(j, mc):
                    m, acc = mc
                    r0, s = scores(e, qa, j)
                    m_new = jnp.maximum(m, jnp.max(s, axis=0, keepdims=True))
                    p = jnp.exp2(s - m_new).astype(bf16)
                    pv = jnp.dot(vT_ref[W * e:W * e + W, pl.ds(r0, TKS)], p, preferred_element_type=f32)
                    return m_new, acc * jnp.exp2(m - m_new) + pv

                m0 = jnp.full((1, tq), -jnp.inf, f32)
                _, acc = lax.fori_loop(0, S // TKS, chunk, (m0, jnp.zeros((W, tq), f32)))
                store_head(pl.multiple_of(40 * pi, 8), e, acc * (1.0 / acc[lrow[e]:lrow[e] + 1]))
            return carry

        lax.fori_loop(0, (H - UPB) // 2, pair_body, 0)
        for u in range(UPB):
            e = u % 2
            qa = q_of((H - UPB) // 2 + u // 2, e)
            buf = UPB * LAST_PAR + u

            def row_max(j, m):
                return jnp.maximum(m, jnp.max(scores(e, qa, j)[1], axis=0, keepdims=True))

            m = lax.fori_loop(0, S // TKS, row_max, jnp.full((1, tq), -jnp.inf, f32))

            def write_p(j, carry):
                r0, s = scores(e, qa, j)
                p = pltpu.bitcast(jnp.exp2(s - m).astype(bf16), u32)
                p_refs[buf][pl.ds(pl.multiple_of(j * (TKS // 2), TKS // 2), TKS // 2), :] = p
                return carry

            lax.fori_loop(0, S // TKS, write_p, 0)

    @pl.when(step == 0)
    def _wait_late():
        for j in range(4):
            late_copy(j).wait()

    @pl.when(step > 0)
    def _wait_prev_out():
        for r in range(tq // OB):
            out_copy(step - 1, r).wait()

    tail()

    @pl.when(step == S // tq - 1)
    def _wait_out():
        for r in range(tq // OB):
            out_copy(step, r).wait()


@jax.jit
def pallas_gated_mix__grouped_kv_mqa__glu_gated_reglu__prompt_kernel(
    A_x: jax.Array,
    A_wq: jax.Array,
    A_wk: jax.Array,
    A_wv: jax.Array,
    A_wo: jax.Array,
    B_x: jax.Array,
    B_W_gate: jax.Array,
    B_W_up: jax.Array,
    B_W_down: jax.Array,
    gate_w: jax.Array,
):
    del B_x
    hbm = pl.BlockSpec(memory_space=pl.ANY)
    out = pl.pallas_call(
        _kernel,
        grid=(S // TQ,),
        in_specs=[hbm] * 9,
        out_specs=hbm,
        out_shape=jax.ShapeDtypeStruct((S, D), bf16),
        scratch_shapes=[
            pltpu.VMEM((S, D), bf16),
            pltpu.VMEM((D, D), bf16),
            pltpu.VMEM((DH, D), bf16),
            pltpu.VMEM((DH, D), bf16),
            pltpu.VMEM((D, D), bf16),
            pltpu.VMEM((D, F), bf16),
            pltpu.VMEM((D, F), bf16),
            pltpu.VMEM((F, D), bf16),
            pltpu.VMEM((D // 128, 128), bf16),
            pltpu.SemaphoreType.DMA((NXC + 8,)),
            pltpu.VMEM((2, S, W), bf16),
            pltpu.VMEM((2 * W, S), f32),
            pltpu.VMEM((D, D), bf16),
            pltpu.VMEM((D, TQ), f32),
            pltpu.VMEM((D, TQ), f32),
            pltpu.VMEM((sum(VU), DH * 128), f32),
            pltpu.VMEM((UPB, DH, 8, TQ), f32),
            pltpu.VMEM((UPB, 8, TQ), f32),
            pltpu.SMEM((1,), f32),
            pltpu.VMEM((TQ, F), bf16),
            pltpu.VMEM((TQ, D), bf16),
            pltpu.SemaphoreType.DMA((TQ // OB,)),
        ] + [pltpu.VMEM((S // 2, TQ), u32)] * (2 * UPB),
        compiler_params=pltpu.CompilerParams(
            dimension_semantics=("arbitrary",), vmem_limit_bytes=120 * 1024 * 1024),
    )(A_x.reshape(S, D), A_wq, A_wk.T, A_wv.T, A_wo, B_W_gate, B_W_up, B_W_down, gate_w.reshape(D // 128, 128))
    return out.reshape(1, S, D)
```

```python
import jax
import jax.numpy as jnp
from jax import lax
import jax.experimental.pallas as pl
import jax.experimental.pallas.tpu as pltpu

S, D, H, DH, F = 2048, 640, 32, 20, 1536
W = 24
LOG2E = 1.4426950408889634
f32, bf16, u32 = jnp.float32, jnp.bfloat16, jnp.uint32
NT = (((1,), (1,)), ((), ()))
TK = 128
NC = S // TK
SCORE_BOUND = 60.0
V_HI = 2.0 ** 40
V_LO = 2.0 ** -30


def make_kernel(tq, nxc, vr, vr0, lead, upb, tks, fb, rb, ob, wq_first, late_at, nocse, joint, qb_at, vlast, pace, qsplit, dsplit, hold, hold_n, qsplit0, dsplit0, qb_at0, tie0, tie1):
    xc = S // nxc
    nbody = H // upb
    nvmax = max(sum(vr), sum(vr0))
    last_par = (nbody - 1) % 2

    def vcfg(v):
        nv = sum(v)
        ngroups = nv // 8
        gps = [((c + 1) * ngroups) // vlast - (c * ngroups) // vlast if c < vlast else 0 for c in range(NC)]
        tpos = {}
        if pace and ngroups:
            nrows = [TK - v[c] for c in range(NC)]
            R = [sum(nrows[:c]) for c in range(NC + 1)]
            gps = [0] * NC
            for g in range(ngroups):
                pos = (g * R[vlast]) // ngroups
                c = max(cc for cc in range(NC) if R[cc] <= pos)
                gps[c] += 1
                tpos[g] = ((pos - R[c]) // 8) * 8
        return dict(tpos=tpos, vr=v, nv=nv, blk_row=[c * TK + 16 * b for c in range(NC) for b in range(v[c] // 16)],
                    glo=[sum(gps[:c]) for c in range(NC + 1)])

    vu = [max(a, b) for a, b in zip(vr, vr0)]
    kbo = [sum(vu[:c]) for c in range(NC + 1)]
    cfg_loop, cfg_first = vcfg(vr), vcfg(vr0)

    def kb_row(key_row):
        c, r = divmod(key_row, TK)
        return kbo[c] + r

    def kernel(x_hbm, wq_hbm, wkT_hbm, wvT_hbm, wo_hbm, wg_hbm, wu_hbm, wd_hbm, gw_hbm,
               o_hbm,
               x_ref, wq_ref, wkT_ref, wvT_ref, wo_ref, wg_ref, wu_ref, wd_ref, gw_ref, sems,
               k_ref, vT_ref, wqT_ref, qT_ref, oT_ref, kb_ref, qb0_ref, qb1_ref, qb2_ref, tok_ref, stat_ref, h_ref, ob_ref, osems, zs_ref, *p_refs):
        step = pl.program_id(0)
        qb_refs = (qb0_ref, qb1_ref, qb2_ref)

        def x_copy(j):
            return pltpu.make_async_copy(x_hbm.at[pl.ds(j * xc, xc)], x_ref.at[pl.ds(j * xc, xc)], sems.at[j])

        small = [(wkT_hbm, wkT_ref), (wvT_hbm, wvT_ref), (gw_hbm, gw_ref), (wq_hbm, wq_ref)]
        late = [(wg_hbm, wg_ref), (wu_hbm, wu_ref), (wd_hbm, wd_ref), (wo_hbm, wo_ref)]

        def small_copy(j):
            return pltpu.make_async_copy(small[j][0], small[j][1], sems.at[nxc + j])

        def late_copy(j):
            return pltpu.make_async_copy(late[j][0], late[j][1], sems.at[nxc + 4 + j])

        def out_copy(s, r):
            return pltpu.make_async_copy(ob_ref.at[pl.ds(r * ob, ob)],
                                         o_hbm.at[pl.ds(pl.multiple_of(s * tq + r * ob, ob), ob)], osems.at[r])

        @pl.when(step == 0)
        def _prologue():
            small_copy(0).start()
            small_copy(1).start()
            for j in range(128):
                zs_ref[j] = 0
            if wq_first:
                small_copy(3).start()
            for j in range(nxc):
                x_copy(j).start()
            if not wq_first:
                small_copy(3).start()
            small_copy(2).start()
            if late_at < 0:
                for j in range(4):
                    late_copy(j).start()
            small_copy(0).wait()
            small_copy(1).wait()
            r = lax.broadcasted_iota(jnp.int32, (2 * W, DH), 0)
            c = lax.broadcasted_iota(jnp.int32, (2 * W, DH), 1)
            Rk = jnp.where(r == c, 1.0, 0.0).astype(bf16)
            Rv = jnp.where(r == c + W, 1.0, 0.0).astype(bf16)
            wkvT = (jnp.dot(Rk, wkT_ref[...], preferred_element_type=f32)
                    + jnp.dot(Rv, wvT_ref[...], preferred_element_type=f32)).astype(bf16)
            if wq_first:
                small_copy(3).wait()
                wqT_ref[...] = wq_ref[...].astype(f32).T.astype(bf16)
            row = lax.broadcasted_iota(jnp.int32, (W, xc), 0)
            r = lax.broadcasted_iota(jnp.int32, (W, DH * 128), 0)
            c = lax.broadcasted_iota(jnp.int32, (W, DH * 128), 1)
            E = jnp.where(r == c // 128, 1.0, 0.0).astype(bf16)
            kmax = None
            vmax = None
            for j in range(nxc):
                x_copy(j).wait()
                if j == late_at:
                    for jj in range(4):
                        late_copy(jj).start()
                rows = pl.ds(j * xc, xc)
                kvT = lax.dot_general(wkvT, x_ref[rows, :], NT, preferred_element_type=f32)
                kvT = kvT.astype(bf16).astype(f32)
                kT, vT = kvT[0:W], kvT[W:2 * W]
                am = jnp.abs(kvT)
                kmax = am[0:W] if kmax is None else jnp.maximum(kmax, am[0:W])
                vmax = am[W:2 * W] if vmax is None else jnp.maximum(vmax, am[W:2 * W])
                vT_ref[0:W, rows] = jnp.where(row == 20, 1.0, vT)
                vT_ref[W:2 * W, rows] = jnp.where(row == 0, 1.0, pltpu.roll(vT, 4, 0))
                kk = jnp.concatenate([kT, jnp.zeros((8, xc), f32), pltpu.roll(kT, 4, 0), jnp.zeros((72, xc), f32)], axis=0)
                k4 = kk.T
                k0 = k4[:, 0:W].astype(bf16)
                k_ref[0, rows, :] = k0
                k_ref[1, rows, :] = k4[:, 32:32 + W].astype(bf16)
                if nvmax:
                    cs = [c for c in range(j * xc // TK, (j + 1) * xc // TK) if vu[c]]
                    ksel = jnp.concatenate([k0[c * TK - j * xc:c * TK - j * xc + vu[c]] for c in cs], axis=0)
                    kb_ref[pl.ds(kbo[cs[0]], ksel.shape[0]), :] = jnp.dot(ksel, E, preferred_element_type=f32)
            vmx = jnp.max(vmax)
            v_ok = jnp.logical_and(vmx <= V_HI, vmx >= V_LO)
            stat_ref[0] = jnp.where(v_ok, jnp.max(kmax) * (DH * 1.02), jnp.inf)
            if not wq_first:
                small_copy(3).wait()
                wqT_ref[...] = wq_ref[...].astype(f32).T.astype(bf16)
            small_copy(2).wait()

        row0 = pl.multiple_of(step * tq, tq)
        xb = x_ref[pl.ds(row0, tq), :]
        qT = lax.dot_general(wqT_ref[...], xb, NT, preferred_element_type=f32) * (DH ** -0.5 * LOG2E)
        qT_ref[...] = qT
        qmax = jnp.max(jnp.max(jnp.abs(qT).reshape(D // 8, 8, tq), axis=0))
        fast = qmax * stat_ref[0] <= SCORE_BOUND

        lrow = (20, 0)

        def mult(v, k):
            return v if isinstance(v, int) else pl.multiple_of(v, k)

        def store_head(base, e, o):
            if e == 0:
                oT_ref[pl.ds(base, W), :] = o
            else:
                r8 = lax.broadcasted_iota(jnp.int32, (8, tq), 0)
                oT_ref[pl.ds(base + 16, 8), :] = jnp.where(r8 < 4, oT_ref[pl.ds(base + 16, 8), :], o[0:8])
                oT_ref[pl.ds(base + 24, 16), :] = o[8:24]

        def build_qb(gi, par, u):
            e = u % 2
            qwin = qT_ref[pl.ds(mult(20 * upb * gi + 40 * (u // 2) + 16 * e, 8), W), :]
            for d in range(DH):
                qb_refs[par][u, d] = jnp.broadcast_to(qwin[4 * e + d:4 * e + d + 1, :], (8, tq))

        def a_slot(st, cfg, bi, par, u, c):
            e = u % 2
            key = ('A', u)
            buf = upb * par + u
            v, glo, blk_row = cfg['vr'], cfg['glo'], cfg['blk_row']
            first = isinstance(bi, int) and bi == 0
            if key not in st:
                qwin = qT_ref[pl.ds(mult(20 * upb * bi + 40 * (u // 2) + 16 * e, 8), W), :]
                st[key] = dict(qa=qwin.astype(bf16), val=None, half=None)
                if first:
                    build_qb(0, 2, u)
            a = st[key]
            if c == (qb_at0 if first else qb_at):
                nxt = bi + 1 if isinstance(bi, int) else jnp.minimum(bi + 1, nbody - 1)
                build_qb(nxt, 1 - par, u)

            def chain(f):
                a['val'] = f if a['val'] is None else jnp.maximum(a['val'], f)

            lo, n = c * TK + v[c], TK - v[c]
            gl = list(range(glo[c], glo[c + 1]))
            nsp = qsplit if not first else qsplit0
            cuts = [0] + [min(n, 16 * ((n // 16 * (i + 1) + nsp - 1) // nsp)) for i in range(nsp)]
            items = []
            for g in gl:
                dsp = dsplit if not first else dsplit0
                for h in range(dsp):
                    items.append((g, h * DH // dsp, (h + 1) * DH // dsp))
            carry_in = a.get('pend', [])
            items = carry_in + items
            a['pend'] = []
            if hold and c < NC - 1 and len(items) > hold_n:
                a['pend'] = items[hold_n:]
                items = items[:hold_n]
            per = [len(items) * (i + 1) // nsp - len(items) * i // nsp for i in range(nsp)]
            it = 0
            for i in range(nsp):
                r0, r1 = cuts[i], cuts[i + 1]
                if r1 > r0:
                    s = jnp.dot(k_ref[e, pl.ds(lo + r0, r1 - r0), :], a['qa'], preferred_element_type=f32)
                    p_refs[buf][pl.ds((lo + r0) // 2, (r1 - r0) // 2), :] = pltpu.bitcast(jnp.exp2(s).astype(bf16), u32)
                    t0 = (tie0 if first else tie1) % (r1 - r0)
                    t0 = min(t0, r1 - r0 - 8)
                    chain(s[t0:t0 + 8])
                for _ in range(per[i]):
                    g, d0, d1 = items[it]
                    it += 1
                    krow = kb_row(blk_row[g // 2] + 8 * (g % 2))
                    uq = u
                    if nocse and not first:
                        z = zs_ref[(u * 32 + g) % 128]
                        krow = pl.multiple_of(krow + 8 * z, 8)
                        uq = u + z
                    sv = a.get(('sv', g))
                    for d in range(d0, d1):
                        kb = kb_ref[pl.ds(krow, 8), pl.ds(128 * d, 128)]
                        kbt = jnp.concatenate([kb] * (tq // 128), axis=1)
                        t = kbt * qb_refs[2 if first else par][uq, d]
                        sv = t if sv is None else sv + t
                    chain(sv)
                    if d1 < DH:
                        a[('sv', g)] = sv
                        continue
                    a.pop(('sv', g), None)
                    pv = jnp.exp2(sv)
                    if g % 2 == 0:
                        a['half'] = pv
                    else:
                        pu = pltpu.bitcast(jnp.concatenate([a['half'], pv], axis=0).astype(bf16), u32)
                        p_refs[buf][pl.ds(blk_row[g // 2] // 2, 8), :] = pu
            if c == NC - 1:
                tok_ref[u] = a['val']
                del st[key]

        def b_slot(st, bi, par, u, c):
            e = u % 2
            buf = upb * par + u
            key = ('B', u)
            if key not in st:
                st[key] = dict(val=None)
            b = st[key]
            p = pltpu.bitcast(p_refs[buf][pl.ds(c * TK // 2, TK // 2), :], bf16)
            vt = vT_ref[W * e:W * e + W, pl.ds(c * TK, TK)]
            pv = jnp.dot(vt, p, preferred_element_type=f32)
            b['val'] = pv if b['val'] is None else b['val'] + pv
            if c == NC - 1:
                acc = b['val']
                store_head(mult(20 * upb * bi + 40 * (u // 2), 8), e, acc * (1.0 / acc[lrow[e]:lrow[e] + 1]))
                del st[key]

        def body(cfg, ia, para, ib, parb):
            st = {}
            nb = 0
            nt = upb * NC
            for t in range(nt):
                if ia is not None:
                    a_slot(st, cfg, ia, para, t // NC, t % NC)
                if ib is not None:
                    while nb < nt and nb <= t + lead:
                        b_slot(st, ib, parb, nb // NC, nb % NC)
                        nb += 1
            if ib is not None:
                while nb < nt:
                    b_slot(st, ib, parb, nb // NC, nb % NC)
                    nb += 1

        def tail():
            st = {}
            nt = upb * NC
            bq = list(range(nt))

            def b_some(n):
                for _ in range(n):
                    if bq:
                        t = bq.pop(0)
                        b_slot(st, nbody - 1, last_par, t // NC, t % NC)

            nfb = F // fb
            per = -(-nt // (2 * nfb * (tq // rb)))
            for j in range(nfb):
                cols = pl.ds(j * fb, fb)
                for r in range(tq // rb):
                    xr = x_ref[pl.ds(row0 + r * rb, rb), :]
                    gate = jnp.dot(xr, wg_ref[:, cols], preferred_element_type=f32)
                    b_some(per)
                    up = jnp.dot(xr, wu_ref[:, cols], preferred_element_type=f32)
                    b_some(per)
                    h_ref[pl.ds(r * rb, rb), cols] = (jnp.maximum(gate, 0.0) * up).astype(bf16)
            b_some(nt)
            o_all = oT_ref[...].T.astype(bf16)
            gw = gw_ref[...].astype(f32)
            for r in range(tq // ob):
                rows = pl.ds(r * ob, ob)
                a_out = jnp.dot(o_all[r * ob:(r + 1) * ob], wo_ref[...], preferred_element_type=f32)
                b_out = jnp.dot(h_ref[rows, :], wd_ref[...], preferred_element_type=f32)
                xf = x_ref[pl.ds(row0 + r * ob, ob), :].astype(f32)
                la = xf[:, 0:128] * gw[0:1, :]
                for j in range(1, D // 128):
                    la = la + xf[:, 128 * j:128 * (j + 1)] * gw[j:j + 1, :]
                g = jax.nn.sigmoid(jnp.sum(la, axis=-1, keepdims=True))
                ob_ref[rows, :] = (g * a_out + (1.0 - g) * b_out).astype(bf16)
                out_copy(step, r).start()

        body(cfg_first, 0, 0, None, None)

        @pl.when(fast)
        def _fast():
            def loop_body(i, carry):
                @pl.when(i % 2 == 0)
                def _():
                    body(cfg_loop, i + 1, 1, i, 0)

                @pl.when(i % 2 == 1)
                def _():
                    body(cfg_loop, i + 1, 0, i, 1)
                return carry

            lax.fori_loop(0, nbody - 1, loop_body, 0)

        @pl.when(jnp.logical_not(fast))
        def _slow():
            def q_of(pi, e):
                return qT_ref[pl.ds(mult(40 * pi + 16 * e, 8), W), :].astype(bf16)

            def scores(e, qa, j):
                r0 = pl.multiple_of(j * tks, tks)
                return r0, jnp.dot(k_ref[e, pl.ds(r0, tks), :], qa, preferred_element_type=f32)

            def pair_body(pi, carry):
                for e in range(2):
                    qa = q_of(pi, e)

                    def chunk(j, mc):
                        m, acc = mc
                        r0, s = scores(e, qa, j)
                        m_new = jnp.maximum(m, jnp.max(s, axis=0, keepdims=True))
                        p = jnp.exp2(s - m_new).astype(bf16)
                        pv = jnp.dot(vT_ref[W * e:W * e + W, pl.ds(r0, tks)], p, preferred_element_type=f32)
                        return m_new, acc * jnp.exp2(m - m_new) + pv

                    m0 = jnp.full((1, tq), -jnp.inf, f32)
                    _, acc = lax.fori_loop(0, S // tks, chunk, (m0, jnp.zeros((W, tq), f32)))
                    store_head(pl.multiple_of(40 * pi, 8), e, acc * (1.0 / acc[lrow[e]:lrow[e] + 1]))
                return carry

            lax.fori_loop(0, (H - upb) // 2, pair_body, 0)
            for u in range(upb):
                e = u % 2
                qa = q_of((H - upb) // 2 + u // 2, e)
                buf = upb * last_par + u

                def row_max(j, m):
                    return jnp.maximum(m, jnp.max(scores(e, qa, j)[1], axis=0, keepdims=True))

                m = lax.fori_loop(0, S // tks, row_max, jnp.full((1, tq), -jnp.inf, f32))

                def write_p(j, carry):
                    r0, s = scores(e, qa, j)
                    p = pltpu.bitcast(jnp.exp2(s - m).astype(bf16), u32)
                    p_refs[buf][pl.ds(pl.multiple_of(j * (tks // 2), tks // 2), tks // 2), :] = p
                    return carry

                lax.fori_loop(0, S // tks, write_p, 0)

        @pl.when(step == 0)
        def _wait_late():
            for j in range(4):
                late_copy(j).wait()

        @pl.when(step > 0)
        def _wait_prev_out():
            for r in range(tq // ob):
                out_copy(step - 1, r).wait()

        tail()

        @pl.when(step == S // tq - 1)
        def _wait_out():
            for r in range(tq // ob):
                out_copy(step, r).wait()
    return kernel


def build(tq=512, nxc=4, vr=None, vr0=None, lead=-1, upb=4, tks=256, fb=512, rb=128, ob=128, wq_first=0, late_at=-1, nocse=3, joint=0, qb_at=4, vlast=16, pace=0, qsplit=4, dsplit=4, hold=0, hold_n=3, qsplit0=1, dsplit0=1, qb_at0=4, tie0=0, tie1=24):
    if vr is None:
        vr = [16] * 16
    if vr0 is None:
        vr0 = [16] * 16

    def run(A_x, A_wq, A_wk, A_wv, A_wo, B_x, B_W_gate, B_W_up, B_W_down, gate_w):
        x = A_x.reshape(S, D)
        gw = gate_w.reshape(D // 128, 128)
        hbm = pl.BlockSpec(memory_space=pl.ANY)
        nvu = sum(max(a, b) for a, b in zip(vr, vr0))
        out = pl.pallas_call(
            make_kernel(tq, nxc, tuple(vr), tuple(vr0), lead, upb, tks, fb, rb, ob, wq_first, late_at, nocse, joint, qb_at, vlast, pace, qsplit, dsplit, hold, hold_n, qsplit0, dsplit0, qb_at0, tie0, tie1),
            grid=(S // tq,),
            in_specs=[hbm] * 9,
            out_specs=hbm,
            out_shape=jax.ShapeDtypeStruct((S, D), bf16),
            scratch_shapes=[
                pltpu.VMEM((S, D), bf16),
                pltpu.VMEM((D, D), bf16),
                pltpu.VMEM((DH, D), bf16),
                pltpu.VMEM((DH, D), bf16),
                pltpu.VMEM((D, D), bf16),
                pltpu.VMEM((D, F), bf16),
                pltpu.VMEM((D, F), bf16),
                pltpu.VMEM((F, D), bf16),
                pltpu.VMEM((D // 128, 128), bf16),
                pltpu.SemaphoreType.DMA((nxc + 8,)),
                pltpu.VMEM((2, S, W), bf16),
                pltpu.VMEM((2 * W, S), f32),
                pltpu.VMEM((D, D), bf16),
                pltpu.VMEM((D, tq), f32),
                pltpu.VMEM((D, tq), f32),
                pltpu.VMEM((max(nvu, 8), DH * 128), f32),
                pltpu.VMEM((upb, DH, 8, tq), f32),
                pltpu.VMEM((upb, DH, 8, tq), f32),
                pltpu.VMEM((upb, DH, 8, tq), f32),
                pltpu.VMEM((upb, 8, tq), f32),
                pltpu.SMEM((1,), f32),
                pltpu.VMEM((tq, F), bf16),
                pltpu.VMEM((tq, D), bf16),
                pltpu.SemaphoreType.DMA((tq // ob,)),
                pltpu.SMEM((128,), jnp.int32),
            ] + [pltpu.VMEM((S // 2, tq), u32)] * (2 * upb),
            compiler_params=pltpu.CompilerParams(
                dimension_semantics=("arbitrary",), vmem_limit_bytes=120 * 1024 * 1024),
        )(x, A_wq, A_wk.T, A_wv.T, A_wo, B_W_gate, B_W_up, B_W_down, gw)
        return out.reshape(1, S, D)
    return jax.jit(run)


_RUN = build()


@jax.jit
def pallas_gated_mix__grouped_kv_mqa__glu_gated_reglu__prompt_kernel(
    A_x: jax.Array,
    A_wq: jax.Array,
    A_wk: jax.Array,
    A_wv: jax.Array,
    A_wo: jax.Array,
    B_x: jax.Array,
    B_W_gate: jax.Array,
    B_W_up: jax.Array,
    B_W_down: jax.Array,
    gate_w: jax.Array,
):
    return _RUN(A_x, A_wq, A_wk, A_wv, A_wo, B_x, B_W_gate, B_W_up, B_W_down, gate_w)
```

```python
import jax
import jax.numpy as jnp
from jax import lax
import jax.experimental.pallas as pl
import jax.experimental.pallas.tpu as pltpu

S, D, H, DH, F = 2048, 640, 32, 20, 1536
W = 24
LOG2E = 1.4426950408889634
f32, bf16, u32 = jnp.float32, jnp.bfloat16, jnp.uint32
NT = (((1,), (1,)), ((), ()))
TK = 128
NC = S // TK
SCORE_BOUND = 60.0
V_HI = 2.0 ** 40
V_LO = 2.0 ** -30


def make_kernel(tq, nxc, vr, vr0, lead, upb, tks, fb, rb, ob, wq_first, late_at, nocse, joint, qb_at, vlast, pace, qsplit, dsplit, hold, hold_n, qsplit0, dsplit0, qb_at0, tie0, tie1):
    xc = S // nxc
    nbody = H // upb
    nvmax = max(sum(vr), sum(vr0))
    last_par = (nbody - 1) % 2

    def vcfg(v):
        nv = sum(v)
        ngroups = nv // 8
        gps = [((c + 1) * ngroups) // vlast - (c * ngroups) // vlast if c < vlast else 0 for c in range(NC)]
        tpos = {}
        if pace and ngroups:
            nrows = [TK - v[c] for c in range(NC)]
            R = [sum(nrows[:c]) for c in range(NC + 1)]
            gps = [0] * NC
            for g in range(ngroups):
                pos = (g * R[vlast]) // ngroups
                c = max(cc for cc in range(NC) if R[cc] <= pos)
                gps[c] += 1
                tpos[g] = ((pos - R[c]) // 8) * 8
        return dict(tpos=tpos, vr=v, nv=nv, blk_row=[c * TK + 16 * b for c in range(NC) for b in range(v[c] // 16)],
                    glo=[sum(gps[:c]) for c in range(NC + 1)])

    vu = [max(a, b) for a, b in zip(vr, vr0)]
    kbo = [sum(vu[:c]) for c in range(NC + 1)]
    cfg_loop, cfg_first = vcfg(vr), vcfg(vr0)

    def kb_row(key_row):
        c, r = divmod(key_row, TK)
        return kbo[c] + r

    def kernel(x_hbm, wq_hbm, wkT_hbm, wvT_hbm, wo_hbm, wg_hbm, wu_hbm, wd_hbm, gw_hbm,
               o_hbm,
               x_ref, wq_ref, wkT_ref, wvT_ref, wo_ref, wg_ref, wu_ref, wd_ref, gw_ref, sems,
               k_ref, vT_ref, wqT_ref, qT_ref, oT_ref, kb_ref, qb0_ref, qb1_ref, qb2_ref, tok_ref, stat_ref, h_ref, ob_ref, osems, zs_ref, *p_refs):
        step = pl.program_id(0)
        qb_refs = (qb0_ref, qb1_ref, qb2_ref)

        def x_copy(j):
            return pltpu.make_async_copy(x_hbm.at[pl.ds(j * xc, xc)], x_ref.at[pl.ds(j * xc, xc)], sems.at[j])

        small = [(wkT_hbm, wkT_ref), (wvT_hbm, wvT_ref), (gw_hbm, gw_ref), (wq_hbm, wq_ref)]
        late = [(wg_hbm, wg_ref), (wu_hbm, wu_ref), (wd_hbm, wd_ref), (wo_hbm, wo_ref)]

        def small_copy(j):
            return pltpu.make_async_copy(small[j][0], small[j][1], sems.at[nxc + j])

        def late_copy(j):
            return pltpu.make_async_copy(late[j][0], late[j][1], sems.at[nxc + 4 + j])

        def out_copy(s, r):
            return pltpu.make_async_copy(ob_ref.at[pl.ds(r * ob, ob)],
                                         o_hbm.at[pl.ds(pl.multiple_of(s * tq + r * ob, ob), ob)], osems.at[r])

        @pl.when(step == 0)
        def _prologue():
            small_copy(0).start()
            small_copy(1).start()
            for j in range(128):
                zs_ref[j] = 0
            if wq_first:
                small_copy(3).start()
            for j in range(nxc):
                x_copy(j).start()
            if not wq_first:
                small_copy(3).start()
            small_copy(2).start()
            if late_at < 0:
                for j in range(4):
                    late_copy(j).start()
            small_copy(0).wait()
            small_copy(1).wait()
            r = lax.broadcasted_iota(jnp.int32, (2 * W, DH), 0)
            c = lax.broadcasted_iota(jnp.int32, (2 * W, DH), 1)
            Rk = jnp.where(r == c, 1.0, 0.0).astype(bf16)
            Rv = jnp.where(r == c + W, 1.0, 0.0).astype(bf16)
            wkvT = (jnp.dot(Rk, wkT_ref[...], preferred_element_type=f32)
                    + jnp.dot(Rv, wvT_ref[...], preferred_element_type=f32)).astype(bf16)
            if wq_first:
                small_copy(3).wait()
                wqT_ref[...] = wq_ref[...].astype(f32).T.astype(bf16)
            row = lax.broadcasted_iota(jnp.int32, (W, xc), 0)
            r = lax.broadcasted_iota(jnp.int32, (W, DH * 128), 0)
            c = lax.broadcasted_iota(jnp.int32, (W, DH * 128), 1)
            E = jnp.where(r == c // 128, 1.0, 0.0).astype(bf16)
            kmax = None
            vmax = None
            for j in range(nxc):
                x_copy(j).wait()
                if j == late_at:
                    for jj in range(4):
                        late_copy(jj).start()
                rows = pl.ds(j * xc, xc)
                kvT = lax.dot_general(wkvT, x_ref[rows, :], NT, preferred_element_type=f32)
                kvT = kvT.astype(bf16).astype(f32)
                kT, vT = kvT[0:W], kvT[W:2 * W]
                am = jnp.abs(kvT)
                kmax = am[0:W] if kmax is None else jnp.maximum(kmax, am[0:W])
                vmax = am[W:2 * W] if vmax is None else jnp.maximum(vmax, am[W:2 * W])
                vT_ref[0:W, rows] = jnp.where(row == 20, 1.0, vT)
                vT_ref[W:2 * W, rows] = jnp.where(row == 0, 1.0, pltpu.roll(vT, 4, 0))
                kk = jnp.concatenate([kT, jnp.zeros((8, xc), f32), pltpu.roll(kT, 4, 0), jnp.zeros((72, xc), f32)], axis=0)
                k4 = kk.T
                k0 = k4[:, 0:W].astype(bf16)
                prow = pl.ds(j * xc // 2, xc // 2)
                k_ref[0, prow, :] = pltpu.bitcast(k0, u32)
                k_ref[1, prow, :] = pltpu.bitcast(k4[:, 32:32 + W].astype(bf16), u32)
                if nvmax:
                    cs = [c for c in range(j * xc // TK, (j + 1) * xc // TK) if vu[c]]
                    ksel = jnp.concatenate([k0[c * TK - j * xc:c * TK - j * xc + vu[c]] for c in cs], axis=0)
                    kb_ref[pl.ds(kbo[cs[0]], ksel.shape[0]), :] = jnp.dot(ksel, E, preferred_element_type=f32)
            vmx = jnp.max(vmax)
            v_ok = jnp.logical_and(vmx <= V_HI, vmx >= V_LO)
            stat_ref[0] = jnp.where(v_ok, jnp.max(kmax) * (DH * 1.02), jnp.inf)
            if not wq_first:
                small_copy(3).wait()
                wqT_ref[...] = wq_ref[...].astype(f32).T.astype(bf16)
            small_copy(2).wait()

        row0 = pl.multiple_of(step * tq, tq)
        xb = x_ref[pl.ds(row0, tq), :]
        qT = lax.dot_general(wqT_ref[...], xb, NT, preferred_element_type=f32) * (DH ** -0.5 * LOG2E)
        qT_ref[...] = qT
        qmax = jnp.max(jnp.max(jnp.abs(qT).reshape(D // 8, 8, tq), axis=0))
        fast = qmax * stat_ref[0] <= SCORE_BOUND

        lrow = (20, 0)

        def mult(v, k):
            return v if isinstance(v, int) else pl.multiple_of(v, k)

        def store_head(base, e, o):
            if e == 0:
                oT_ref[pl.ds(base, W), :] = o
            else:
                r8 = lax.broadcasted_iota(jnp.int32, (8, tq), 0)
                oT_ref[pl.ds(base + 16, 8), :] = jnp.where(r8 < 4, oT_ref[pl.ds(base + 16, 8), :], o[0:8])
                oT_ref[pl.ds(base + 24, 16), :] = o[8:24]

        def build_qb(gi, par, u):
            e = u % 2
            qwin = qT_ref[pl.ds(mult(20 * upb * gi + 40 * (u // 2) + 16 * e, 8), W), :]
            for d in range(DH):
                qb_refs[par][u, d] = jnp.broadcast_to(qwin[4 * e + d:4 * e + d + 1, :], (8, tq))

        def a_slot(st, cfg, bi, par, u, c):
            e = u % 2
            key = ('A', u)
            buf = upb * par + u
            v, glo, blk_row = cfg['vr'], cfg['glo'], cfg['blk_row']
            first = isinstance(bi, int) and bi == 0
            if key not in st:
                qwin = qT_ref[pl.ds(mult(20 * upb * bi + 40 * (u // 2) + 16 * e, 8), W), :]
                st[key] = dict(qa=qwin.astype(bf16), val=None, half=None)
                if first:
                    build_qb(0, 2, u)
            a = st[key]
            if c == (qb_at0 if first else qb_at):
                nxt = bi + 1 if isinstance(bi, int) else jnp.minimum(bi + 1, nbody - 1)
                build_qb(nxt, 1 - par, u)

            def chain(f):
                a['val'] = f if a['val'] is None else jnp.maximum(a['val'], f)

            lo, n = c * TK + v[c], TK - v[c]
            gl = list(range(glo[c], glo[c + 1]))
            nsp = qsplit if not first else qsplit0
            cuts = [0] + [min(n, 16 * ((n // 16 * (i + 1) + nsp - 1) // nsp)) for i in range(nsp)]
            items = []
            for g in gl:
                dsp = dsplit if not first else dsplit0
                for h in range(dsp):
                    items.append((g, h * DH // dsp, (h + 1) * DH // dsp))
            carry_in = a.get('pend', [])
            items = carry_in + items
            a['pend'] = []
            if hold and c < NC - 1 and len(items) > hold_n:
                a['pend'] = items[hold_n:]
                items = items[:hold_n]
            per = [len(items) * (i + 1) // nsp - len(items) * i // nsp for i in range(nsp)]
            it = 0
            for i in range(nsp):
                r0, r1 = cuts[i], cuts[i + 1]
                if r1 > r0:
                    kk_ = pltpu.bitcast(k_ref[e, pl.ds((lo + r0) // 2, (r1 - r0) // 2), :], bf16)
                    s = jnp.dot(kk_, a['qa'], preferred_element_type=f32)
                    p_refs[buf][pl.ds((lo + r0) // 2, (r1 - r0) // 2), :] = pltpu.bitcast(jnp.exp2(s).astype(bf16), u32)
                    t0 = (tie0 if first else tie1) % (r1 - r0)
                    t0 = min(t0, r1 - r0 - 8)
                    chain(s[t0:t0 + 8])
                for _ in range(per[i]):
                    g, d0, d1 = items[it]
                    it += 1
                    krow = kb_row(blk_row[g // 2] + 8 * (g % 2))
                    uq = u
                    if nocse and not first:
                        z = zs_ref[(u * 32 + g) % 128]
                        krow = pl.multiple_of(krow + 8 * z, 8)
                        uq = u + z
                    sv = a.get(('sv', g))
                    for d in range(d0, d1):
                        kb = kb_ref[pl.ds(krow, 8), pl.ds(128 * d, 128)]
                        kbt = jnp.concatenate([kb] * (tq // 128), axis=1)
                        t = kbt * qb_refs[2 if first else par][uq, d]
                        sv = t if sv is None else sv + t
                    chain(sv)
                    if d1 < DH:
                        a[('sv', g)] = sv
                        continue
                    a.pop(('sv', g), None)
                    pv = jnp.exp2(sv)
                    if g % 2 == 0:
                        a['half'] = pv
                    else:
                        pu = pltpu.bitcast(jnp.concatenate([a['half'], pv], axis=0).astype(bf16), u32)
                        p_refs[buf][pl.ds(blk_row[g // 2] // 2, 8), :] = pu
            if c == NC - 1:
                tok_ref[u] = a['val']
                del st[key]

        def b_slot(st, bi, par, u, c):
            e = u % 2
            buf = upb * par + u
            key = ('B', u)
            if key not in st:
                st[key] = dict(val=None)
            b = st[key]
            p = pltpu.bitcast(p_refs[buf][pl.ds(c * TK // 2, TK // 2), :], bf16)
            vt = vT_ref[W * e:W * e + W, pl.ds(c * TK, TK)]
            pv = jnp.dot(vt, p, preferred_element_type=f32)
            b['val'] = pv if b['val'] is None else b['val'] + pv
            if c == NC - 1:
                acc = b['val']
                store_head(mult(20 * upb * bi + 40 * (u // 2), 8), e, acc * (1.0 / acc[lrow[e]:lrow[e] + 1]))
                del st[key]

        def body(cfg, ia, para, ib, parb):
            st = {}
            nb = 0
            nt = upb * NC
            for t in range(nt):
                if ia is not None:
                    a_slot(st, cfg, ia, para, t // NC, t % NC)
                if ib is not None:
                    while nb < nt and nb <= t + lead:
                        b_slot(st, ib, parb, nb // NC, nb % NC)
                        nb += 1
            if ib is not None:
                while nb < nt:
                    b_slot(st, ib, parb, nb // NC, nb % NC)
                    nb += 1

        def tail():
            st = {}
            nt = upb * NC
            bq = list(range(nt))

            def b_some(n):
                for _ in range(n):
                    if bq:
                        t = bq.pop(0)
                        b_slot(st, nbody - 1, last_par, t // NC, t % NC)

            nfb = F // fb
            per = -(-nt // (2 * nfb * (tq // rb)))
            for j in range(nfb):
                cols = pl.ds(j * fb, fb)
                for r in range(tq // rb):
                    xr = x_ref[pl.ds(row0 + r * rb, rb), :]
                    gate = jnp.dot(xr, wg_ref[:, cols], preferred_element_type=f32)
                    b_some(per)
                    up = jnp.dot(xr, wu_ref[:, cols], preferred_element_type=f32)
                    b_some(per)
                    h_ref[pl.ds(r * rb, rb), cols] = (jnp.maximum(gate, 0.0) * up).astype(bf16)
            b_some(nt)
            o_all = oT_ref[...].T.astype(bf16)
            gw = gw_ref[...].astype(f32)
            for r in range(tq // ob):
                rows = pl.ds(r * ob, ob)
                a_out = jnp.dot(o_all[r * ob:(r + 1) * ob], wo_ref[...], preferred_element_type=f32)
                b_out = jnp.dot(h_ref[rows, :], wd_ref[...], preferred_element_type=f32)
                xf = x_ref[pl.ds(row0 + r * ob, ob), :].astype(f32)
                la = xf[:, 0:128] * gw[0:1, :]
                for j in range(1, D // 128):
                    la = la + xf[:, 128 * j:128 * (j + 1)] * gw[j:j + 1, :]
                g = jax.nn.sigmoid(jnp.sum(la, axis=-1, keepdims=True))
                ob_ref[rows, :] = (g * a_out + (1.0 - g) * b_out).astype(bf16)
                out_copy(step, r).start()

        body(cfg_first, 0, 0, None, None)

        @pl.when(fast)
        def _fast():
            def loop_body(i, carry):
                @pl.when(i % 2 == 0)
                def _():
                    body(cfg_loop, i + 1, 1, i, 0)

                @pl.when(i % 2 == 1)
                def _():
                    body(cfg_loop, i + 1, 0, i, 1)
                return carry

            lax.fori_loop(0, nbody - 1, loop_body, 0)

        @pl.when(jnp.logical_not(fast))
        def _slow():
            def q_of(pi, e):
                return qT_ref[pl.ds(mult(40 * pi + 16 * e, 8), W), :].astype(bf16)

            def scores(e, qa, j):
                r0 = pl.multiple_of(j * tks, tks)
                kk_ = pltpu.bitcast(k_ref[e, pl.ds(pl.multiple_of(j * (tks // 2), tks // 2), tks // 2), :], bf16)
                return r0, jnp.dot(kk_, qa, preferred_element_type=f32)

            def pair_body(pi, carry):
                for e in range(2):
                    qa = q_of(pi, e)

                    def chunk(j, mc):
                        m, acc = mc
                        r0, s = scores(e, qa, j)
                        m_new = jnp.maximum(m, jnp.max(s, axis=0, keepdims=True))
                        p = jnp.exp2(s - m_new).astype(bf16)
                        pv = jnp.dot(vT_ref[W * e:W * e + W, pl.ds(r0, tks)], p, preferred_element_type=f32)
                        return m_new, acc * jnp.exp2(m - m_new) + pv

                    m0 = jnp.full((1, tq), -jnp.inf, f32)
                    _, acc = lax.fori_loop(0, S // tks, chunk, (m0, jnp.zeros((W, tq), f32)))
                    store_head(pl.multiple_of(40 * pi, 8), e, acc * (1.0 / acc[lrow[e]:lrow[e] + 1]))
                return carry

            lax.fori_loop(0, (H - upb) // 2, pair_body, 0)
            for u in range(upb):
                e = u % 2
                qa = q_of((H - upb) // 2 + u // 2, e)
                buf = upb * last_par + u

                def row_max(j, m):
                    return jnp.maximum(m, jnp.max(scores(e, qa, j)[1], axis=0, keepdims=True))

                m = lax.fori_loop(0, S // tks, row_max, jnp.full((1, tq), -jnp.inf, f32))

                def write_p(j, carry):
                    r0, s = scores(e, qa, j)
                    p = pltpu.bitcast(jnp.exp2(s - m).astype(bf16), u32)
                    p_refs[buf][pl.ds(pl.multiple_of(j * (tks // 2), tks // 2), tks // 2), :] = p
                    return carry

                lax.fori_loop(0, S // tks, write_p, 0)

        @pl.when(step == 0)
        def _wait_late():
            for j in range(4):
                late_copy(j).wait()

        @pl.when(step > 0)
        def _wait_prev_out():
            for r in range(tq // ob):
                out_copy(step - 1, r).wait()

        tail()

        @pl.when(step == S // tq - 1)
        def _wait_out():
            for r in range(tq // ob):
                out_copy(step, r).wait()
    return kernel


def build(tq=512, nxc=4, vr=None, vr0=None, lead=-1, upb=4, tks=256, fb=512, rb=128, ob=128, wq_first=0, late_at=-1, nocse=3, joint=0, qb_at=4, vlast=16, pace=0, qsplit=4, dsplit=4, hold=0, hold_n=3, qsplit0=1, dsplit0=1, qb_at0=4, tie0=0, tie1=24):
    if vr is None:
        vr = [16] * 16
    if vr0 is None:
        vr0 = [16] * 16

    def run(A_x, A_wq, A_wk, A_wv, A_wo, B_x, B_W_gate, B_W_up, B_W_down, gate_w):
        x = A_x.reshape(S, D)
        gw = gate_w.reshape(D // 128, 128)
        hbm = pl.BlockSpec(memory_space=pl.ANY)
        nvu = sum(max(a, b) for a, b in zip(vr, vr0))
        out = pl.pallas_call(
            make_kernel(tq, nxc, tuple(vr), tuple(vr0), lead, upb, tks, fb, rb, ob, wq_first, late_at, nocse, joint, qb_at, vlast, pace, qsplit, dsplit, hold, hold_n, qsplit0, dsplit0, qb_at0, tie0, tie1),
            grid=(S // tq,),
            in_specs=[hbm] * 9,
            out_specs=hbm,
            out_shape=jax.ShapeDtypeStruct((S, D), bf16),
            scratch_shapes=[
                pltpu.VMEM((S, D), bf16),
                pltpu.VMEM((D, D), bf16),
                pltpu.VMEM((DH, D), bf16),
                pltpu.VMEM((DH, D), bf16),
                pltpu.VMEM((D, D), bf16),
                pltpu.VMEM((D, F), bf16),
                pltpu.VMEM((D, F), bf16),
                pltpu.VMEM((F, D), bf16),
                pltpu.VMEM((D // 128, 128), bf16),
                pltpu.SemaphoreType.DMA((nxc + 8,)),
                pltpu.VMEM((2, S // 2, W), u32),
                pltpu.VMEM((2 * W, S), f32),
                pltpu.VMEM((D, D), bf16),
                pltpu.VMEM((D, tq), f32),
                pltpu.VMEM((D, tq), f32),
                pltpu.VMEM((max(nvu, 8), DH * 128), f32),
                pltpu.VMEM((upb, DH, 8, tq), f32),
                pltpu.VMEM((upb, DH, 8, tq), f32),
                pltpu.VMEM((upb, DH, 8, tq), f32),
                pltpu.VMEM((upb, 8, tq), f32),
                pltpu.SMEM((1,), f32),
                pltpu.VMEM((tq, F), bf16),
                pltpu.VMEM((tq, D), bf16),
                pltpu.SemaphoreType.DMA((tq // ob,)),
                pltpu.SMEM((128,), jnp.int32),
            ] + [pltpu.VMEM((S // 2, tq), u32)] * (2 * upb),
            compiler_params=pltpu.CompilerParams(
                dimension_semantics=("arbitrary",), vmem_limit_bytes=120 * 1024 * 1024),
        )(x, A_wq, A_wk.T, A_wv.T, A_wo, B_W_gate, B_W_up, B_W_down, gw)
        return out.reshape(1, S, D)
    return jax.jit(run)


_RUN = build(tie1=8)


@jax.jit
def pallas_gated_mix__grouped_kv_mqa__glu_gated_reglu__prompt_kernel(
    A_x: jax.Array,
    A_wq: jax.Array,
    A_wk: jax.Array,
    A_wv: jax.Array,
    A_wo: jax.Array,
    B_x: jax.Array,
    B_W_gate: jax.Array,
    B_W_up: jax.Array,
    B_W_down: jax.Array,
    gate_w: jax.Array,
):
    return _RUN(A_x, A_wq, A_wk, A_wv, A_wo, B_x, B_W_gate, B_W_up, B_W_down, gate_w)
```

```python
import jax
import jax.numpy as jnp
from jax import lax
import jax.experimental.pallas as pl
import jax.experimental.pallas.tpu as pltpu

S, D, H, DH, F = 2048, 640, 32, 20, 1536
W = 24
LOG2E = 1.4426950408889634
f32, bf16, u32 = jnp.float32, jnp.bfloat16, jnp.uint32
NT = (((1,), (1,)), ((), ()))

TQ = 512
TK = 128
NC = S // TK
NXC = 4
XC = S // NXC
UPB = 4
NGRP = H // UPB
LAST_PAR = (NGRP - 1) % 2
LEAD = -1
TKS = 256
FB, RB, OB = 512, 128, 128
VR = 16
QSPLIT = 4
DSPLIT = 4
QB_AT = 4
TIE = 8

SCORE_BOUND = 60.0
V_HI = 2.0 ** 40
V_LO = 2.0 ** -30


def _kb_row(c, g):
    return VR * c + 8 * g


def _mult(v, k):
    return v if isinstance(v, int) else pl.multiple_of(v, k)


def _kernel(x_hbm, wq_hbm, wkT_hbm, wvT_hbm, wo_hbm, wg_hbm, wu_hbm, wd_hbm, gw_hbm,
            o_hbm,
            x_ref, wq_ref, wkT_ref, wvT_ref, wo_ref, wg_ref, wu_ref, wd_ref, gw_ref, sems,
            k_ref, vT_ref, wqT_ref, qT_ref, oT_ref, kb_ref, qb0_ref, qb1_ref, qb2_ref, tok_ref, stat_ref,
            h_ref, ob_ref, osems, zs_ref, *p_refs):
    step = pl.program_id(0)
    qb_refs = (qb0_ref, qb1_ref, qb2_ref)
    tq = TQ

    def x_copy(j):
        return pltpu.make_async_copy(x_hbm.at[pl.ds(j * XC, XC)], x_ref.at[pl.ds(j * XC, XC)], sems.at[j])

    small = [(wkT_hbm, wkT_ref), (wvT_hbm, wvT_ref), (gw_hbm, gw_ref), (wq_hbm, wq_ref)]
    late = [(wg_hbm, wg_ref), (wu_hbm, wu_ref), (wd_hbm, wd_ref), (wo_hbm, wo_ref)]

    def small_copy(j):
        return pltpu.make_async_copy(small[j][0], small[j][1], sems.at[NXC + j])

    def late_copy(j):
        return pltpu.make_async_copy(late[j][0], late[j][1], sems.at[NXC + 4 + j])

    def out_copy(s, r):
        return pltpu.make_async_copy(ob_ref.at[pl.ds(r * OB, OB)],
                                     o_hbm.at[pl.ds(pl.multiple_of(s * tq + r * OB, OB), OB)], osems.at[r])

    @pl.when(step == 0)
    def _prologue():
        small_copy(0).start()
        small_copy(1).start()
        for j in range(128):
            zs_ref[j] = 0
        for j in range(NXC):
            x_copy(j).start()
        small_copy(3).start()
        small_copy(2).start()
        for j in range(4):
            late_copy(j).start()
        small_copy(0).wait()
        small_copy(1).wait()
        r = lax.broadcasted_iota(jnp.int32, (2 * W, DH), 0)
        c = lax.broadcasted_iota(jnp.int32, (2 * W, DH), 1)
        Rk = jnp.where(r == c, 1.0, 0.0).astype(bf16)
        Rv = jnp.where(r == c + W, 1.0, 0.0).astype(bf16)
        wkvT = (jnp.dot(Rk, wkT_ref[...], preferred_element_type=f32)
                + jnp.dot(Rv, wvT_ref[...], preferred_element_type=f32)).astype(bf16)
        row = lax.broadcasted_iota(jnp.int32, (W, XC), 0)
        r = lax.broadcasted_iota(jnp.int32, (W, DH * 128), 0)
        c = lax.broadcasted_iota(jnp.int32, (W, DH * 128), 1)
        E = jnp.where(r == c // 128, 1.0, 0.0).astype(bf16)
        kmax = None
        vmax = None
        for j in range(NXC):
            x_copy(j).wait()
            rows = pl.ds(j * XC, XC)
            kvT = lax.dot_general(wkvT, x_ref[rows, :], NT, preferred_element_type=f32)
            kvT = kvT.astype(bf16).astype(f32)
            kT, vT = kvT[0:W], kvT[W:2 * W]
            am = jnp.abs(kvT)
            kmax = am[0:W] if kmax is None else jnp.maximum(kmax, am[0:W])
            vmax = am[W:2 * W] if vmax is None else jnp.maximum(vmax, am[W:2 * W])
            vT_ref[0:W, rows] = jnp.where(row == 20, 1.0, vT)
            vT_ref[W:2 * W, rows] = jnp.where(row == 0, 1.0, pltpu.roll(vT, 4, 0))
            kk = jnp.concatenate([kT, jnp.zeros((8, XC), f32), pltpu.roll(kT, 4, 0), jnp.zeros((72, XC), f32)],
                                 axis=0)
            k4 = kk.T
            k0 = k4[:, 0:W].astype(bf16)
            prow = pl.ds(j * XC // 2, XC // 2)
            k_ref[0, prow, :] = pltpu.bitcast(k0, u32)
            k_ref[1, prow, :] = pltpu.bitcast(k4[:, 32:32 + W].astype(bf16), u32)
            cs = list(range(j * XC // TK, (j + 1) * XC // TK))
            ksel = jnp.concatenate([k0[c * TK - j * XC:c * TK - j * XC + VR] for c in cs], axis=0)
            kb_ref[pl.ds(VR * cs[0], ksel.shape[0]), :] = jnp.dot(ksel, E, preferred_element_type=f32)
        vmx = jnp.max(vmax)
        v_ok = jnp.logical_and(vmx <= V_HI, vmx >= V_LO)
        stat_ref[0] = jnp.where(v_ok, jnp.max(kmax) * (DH * 1.02), jnp.inf)
        small_copy(3).wait()
        wqT_ref[...] = wq_ref[...].astype(f32).T.astype(bf16)
        small_copy(2).wait()

    row0 = pl.multiple_of(step * tq, tq)
    xb = x_ref[pl.ds(row0, tq), :]
    qT = lax.dot_general(wqT_ref[...], xb, NT, preferred_element_type=f32) * (DH ** -0.5 * LOG2E)
    qT_ref[...] = qT
    qmax = jnp.max(jnp.max(jnp.abs(qT).reshape(D // 8, 8, tq), axis=0))
    fast = qmax * stat_ref[0] <= SCORE_BOUND

    lrow = (20, 0)

    def store_head(base, e, o):
        if e == 0:
            oT_ref[pl.ds(base, W), :] = o
        else:
            r8 = lax.broadcasted_iota(jnp.int32, (8, tq), 0)
            oT_ref[pl.ds(base + 16, 8), :] = jnp.where(r8 < 4, oT_ref[pl.ds(base + 16, 8), :], o[0:8])
            oT_ref[pl.ds(base + 24, 16), :] = o[8:24]

    def build_qb(gi, par, u):
        e = u % 2
        qwin = qT_ref[pl.ds(_mult(20 * UPB * gi + 40 * (u // 2) + 16 * e, 8), W), :]
        for d in range(DH):
            qb_refs[par][u, d] = jnp.broadcast_to(qwin[4 * e + d:4 * e + d + 1, :], (8, tq))

    def a_slot(st, bi, par, u, c):
        e = u % 2
        key = ('A', u)
        buf = UPB * par + u
        first = isinstance(bi, int) and bi == 0
        if key not in st:
            qwin = qT_ref[pl.ds(_mult(20 * UPB * bi + 40 * (u // 2) + 16 * e, 8), W), :]
            st[key] = dict(qa=qwin.astype(bf16), val=None, half=None)
            if first:
                build_qb(0, 2, u)
        a = st[key]
        if c == QB_AT:
            nxt = bi + 1 if isinstance(bi, int) else jnp.minimum(bi + 1, NGRP - 1)
            build_qb(nxt, 1 - par, u)

        def chain(f):
            a['val'] = f if a['val'] is None else jnp.maximum(a['val'], f)

        lo, n = c * TK + VR, TK - VR
        nsp = 1 if first else QSPLIT
        dsp = 1 if first else DSPLIT
        cuts = [0] + [min(n, 16 * ((n // 16 * (i + 1) + nsp - 1) // nsp)) for i in range(nsp)]
        items = [(g, h * DH // dsp, (h + 1) * DH // dsp) for g in range(2) for h in range(dsp)]
        per = [len(items) * (i + 1) // nsp - len(items) * i // nsp for i in range(nsp)]
        it = 0
        for i in range(nsp):
            r0, r1 = cuts[i], cuts[i + 1]
            kk = pltpu.bitcast(k_ref[e, pl.ds((lo + r0) // 2, (r1 - r0) // 2), :], bf16)
            s = jnp.dot(kk, a['qa'], preferred_element_type=f32)
            p_refs[buf][pl.ds((lo + r0) // 2, (r1 - r0) // 2), :] = pltpu.bitcast(jnp.exp2(s).astype(bf16), u32)
            t0 = min((0 if first else TIE) % (r1 - r0), r1 - r0 - 8)
            chain(s[t0:t0 + 8])
            for _ in range(per[i]):
                g, d0, d1 = items[it]
                it += 1
                krow = _kb_row(c, g)
                uq = u
                if not first:
                    z = zs_ref[(u * 32 + 2 * c + g) % 128]
                    krow = pl.multiple_of(krow + 8 * z, 8)
                    uq = u + z
                sv = a.get(('sv', g))
                for d in range(d0, d1):
                    kb = kb_ref[pl.ds(krow, 8), pl.ds(128 * d, 128)]
                    kbt = jnp.concatenate([kb] * (tq // 128), axis=1)
                    t = kbt * qb_refs[2 if first else par][uq, d]
                    sv = t if sv is None else sv + t
                chain(sv)
                if d1 < DH:
                    a[('sv', g)] = sv
                    continue
                a.pop(('sv', g), None)
                pv = jnp.exp2(sv)
                if g == 0:
                    a['half'] = pv
                else:
                    pu = pltpu.bitcast(jnp.concatenate([a['half'], pv], axis=0).astype(bf16), u32)
                    p_refs[buf][pl.ds(c * TK // 2, 8), :] = pu
        if c == NC - 1:
            tok_ref[u] = a['val']
            del st[key]

    def b_slot(st, bi, par, u, c):
        e = u % 2
        buf = UPB * par + u
        key = ('B', u)
        if key not in st:
            st[key] = dict(val=None)
        b = st[key]
        p = pltpu.bitcast(p_refs[buf][pl.ds(c * TK // 2, TK // 2), :], bf16)
        vt = vT_ref[W * e:W * e + W, pl.ds(c * TK, TK)]
        pv = jnp.dot(vt, p, preferred_element_type=f32)
        b['val'] = pv if b['val'] is None else b['val'] + pv
        if c == NC - 1:
            acc = b['val']
            store_head(_mult(20 * UPB * bi + 40 * (u // 2), 8), e, acc * (1.0 / acc[lrow[e]:lrow[e] + 1]))
            del st[key]

    def body(ia, para, ib, parb):
        st = {}
        nb = 0
        nt = UPB * NC
        for t in range(nt):
            if ia is not None:
                a_slot(st, ia, para, t // NC, t % NC)
            if ib is not None:
                while nb < nt and nb <= t + LEAD:
                    b_slot(st, ib, parb, nb // NC, nb % NC)
                    nb += 1
        if ib is not None:
            while nb < nt:
                b_slot(st, ib, parb, nb // NC, nb % NC)
                nb += 1

    def tail():
        st = {}
        nt = UPB * NC
        bq = list(range(nt))

        def b_some(n):
            for _ in range(n):
                if bq:
                    t = bq.pop(0)
                    b_slot(st, NGRP - 1, LAST_PAR, t // NC, t % NC)

        nfb = F // FB
        per = -(-nt // (2 * nfb * (tq // RB)))
        for j in range(nfb):
            cols = pl.ds(j * FB, FB)
            for r in range(tq // RB):
                xr = x_ref[pl.ds(row0 + r * RB, RB), :]
                gate = jnp.dot(xr, wg_ref[:, cols], preferred_element_type=f32)
                b_some(per)
                up = jnp.dot(xr, wu_ref[:, cols], preferred_element_type=f32)
                b_some(per)
                h_ref[pl.ds(r * RB, RB), cols] = (jnp.maximum(gate, 0.0) * up).astype(bf16)
        b_some(nt)
        o_all = oT_ref[...].T.astype(bf16)
        gw = gw_ref[...].astype(f32)
        for r in range(tq // OB):
            rows = pl.ds(r * OB, OB)
            a_out = jnp.dot(o_all[r * OB:(r + 1) * OB], wo_ref[...], preferred_element_type=f32)
            b_out = jnp.dot(h_ref[rows, :], wd_ref[...], preferred_element_type=f32)
            xf = x_ref[pl.ds(row0 + r * OB, OB), :].astype(f32)
            la = xf[:, 0:128] * gw[0:1, :]
            for j in range(1, D // 128):
                la = la + xf[:, 128 * j:128 * (j + 1)] * gw[j:j + 1, :]
            g = jax.nn.sigmoid(jnp.sum(la, axis=-1, keepdims=True))
            ob_ref[rows, :] = (g * a_out + (1.0 - g) * b_out).astype(bf16)
            out_copy(step, r).start()

    body(0, 0, None, None)

    @pl.when(fast)
    def _fast():
        def loop_body(i, carry):
            @pl.when(i % 2 == 0)
            def _():
                body(i + 1, 1, i, 0)

            @pl.when(i % 2 == 1)
            def _():
                body(i + 1, 0, i, 1)
            return carry

        lax.fori_loop(0, NGRP - 1, loop_body, 0)

    @pl.when(jnp.logical_not(fast))
    def _slow():
        def q_of(pi, e):
            return qT_ref[pl.ds(_mult(40 * pi + 16 * e, 8), W), :].astype(bf16)

        def scores(e, qa, j):
            r0 = pl.multiple_of(j * TKS, TKS)
            kk = pltpu.bitcast(k_ref[e, pl.ds(pl.multiple_of(j * (TKS // 2), TKS // 2), TKS // 2), :], bf16)
            return r0, jnp.dot(kk, qa, preferred_element_type=f32)

        def pair_body(pi, carry):
            for e in range(2):
                qa = q_of(pi, e)

                def chunk(j, mc):
                    m, acc = mc
                    r0, s = scores(e, qa, j)
                    m_new = jnp.maximum(m, jnp.max(s, axis=0, keepdims=True))
                    p = jnp.exp2(s - m_new).astype(bf16)
                    pv = jnp.dot(vT_ref[W * e:W * e + W, pl.ds(r0, TKS)], p, preferred_element_type=f32)
                    return m_new, acc * jnp.exp2(m - m_new) + pv

                m0 = jnp.full((1, tq), -jnp.inf, f32)
                _, acc = lax.fori_loop(0, S // TKS, chunk, (m0, jnp.zeros((W, tq), f32)))
                store_head(pl.multiple_of(40 * pi, 8), e, acc * (1.0 / acc[lrow[e]:lrow[e] + 1]))
            return carry

        lax.fori_loop(0, (H - UPB) // 2, pair_body, 0)
        for u in range(UPB):
            e = u % 2
            qa = q_of((H - UPB) // 2 + u // 2, e)
            buf = UPB * LAST_PAR + u

            def row_max(j, m):
                return jnp.maximum(m, jnp.max(scores(e, qa, j)[1], axis=0, keepdims=True))

            m = lax.fori_loop(0, S // TKS, row_max, jnp.full((1, tq), -jnp.inf, f32))

            def write_p(j, carry):
                r0, s = scores(e, qa, j)
                p = pltpu.bitcast(jnp.exp2(s - m).astype(bf16), u32)
                p_refs[buf][pl.ds(pl.multiple_of(j * (TKS // 2), TKS // 2), TKS // 2), :] = p
                return carry

            lax.fori_loop(0, S // TKS, write_p, 0)

    @pl.when(step == 0)
    def _wait_late():
        for j in range(4):
            late_copy(j).wait()

    @pl.when(step > 0)
    def _wait_prev_out():
        for r in range(tq // OB):
            out_copy(step - 1, r).wait()

    tail()

    @pl.when(step == S // tq - 1)
    def _wait_out():
        for r in range(tq // OB):
            out_copy(step, r).wait()


@jax.jit
def pallas_gated_mix__grouped_kv_mqa__glu_gated_reglu__prompt_kernel(
    A_x: jax.Array,
    A_wq: jax.Array,
    A_wk: jax.Array,
    A_wv: jax.Array,
    A_wo: jax.Array,
    B_x: jax.Array,
    B_W_gate: jax.Array,
    B_W_up: jax.Array,
    B_W_down: jax.Array,
    gate_w: jax.Array,
):
    del B_x
    hbm = pl.BlockSpec(memory_space=pl.ANY)
    out = pl.pallas_call(
        _kernel,
        grid=(S // TQ,),
        in_specs=[hbm] * 9,
        out_specs=hbm,
        out_shape=jax.ShapeDtypeStruct((S, D), bf16),
        scratch_shapes=[
            pltpu.VMEM((S, D), bf16),
            pltpu.VMEM((D, D), bf16),
            pltpu.VMEM((DH, D), bf16),
            pltpu.VMEM((DH, D), bf16),
            pltpu.VMEM((D, D), bf16),
            pltpu.VMEM((D, F), bf16),
            pltpu.VMEM((D, F), bf16),
            pltpu.VMEM((F, D), bf16),
            pltpu.VMEM((D // 128, 128), bf16),
            pltpu.SemaphoreType.DMA((NXC + 8,)),
            pltpu.VMEM((2, S // 2, W), u32),
            pltpu.VMEM((2 * W, S), f32),
            pltpu.VMEM((D, D), bf16),
            pltpu.VMEM((D, TQ), f32),
            pltpu.VMEM((D, TQ), f32),
            pltpu.VMEM((VR * NC, DH * 128), f32),
            pltpu.VMEM((UPB, DH, 8, TQ), f32),
            pltpu.VMEM((UPB, DH, 8, TQ), f32),
            pltpu.VMEM((UPB, DH, 8, TQ), f32),
            pltpu.VMEM((UPB, 8, TQ), f32),
            pltpu.SMEM((1,), f32),
            pltpu.VMEM((TQ, F), bf16),
            pltpu.VMEM((TQ, D), bf16),
            pltpu.SemaphoreType.DMA((TQ // OB,)),
            pltpu.SMEM((128,), jnp.int32),
        ] + [pltpu.VMEM((S // 2, TQ), u32)] * (2 * UPB),
        compiler_params=pltpu.CompilerParams(
            dimension_semantics=("arbitrary",), vmem_limit_bytes=120 * 1024 * 1024),
    )(A_x.reshape(S, D), A_wq, A_wk.T, A_wv.T, A_wo, B_W_gate, B_W_up, B_W_down, gate_w.reshape(D // 128, 128))
    return out.reshape(1, S, D)
```
